```python
import os as _os
_os.environ.setdefault("JAX_PLATFORMS", "cpu")
import jax
import jax.numpy as jnp

def _softmax(x, axis=-1):
    return jax.nn.softmax(x, axis=axis)
def _gelu(x):
    return jax.nn.gelu(x, approximate=True)
def _silu(x):
    return jax.nn.silu(x)
def _sigmoid(x):
    return jax.nn.sigmoid(x)
def _layernorm(x, axis=-1, eps=1e-5):
    m = jnp.mean(x, axis=axis, keepdims=True)
    v = jnp.var(x, axis=axis, keepdims=True)
    return (x - m) / jnp.sqrt(v + eps)
def _scatter_add(tgt, idx, src, axis=0):
    return tgt.at[idx].add(src)
def _segment_sum(src, seg, n):
    return jax.ops.segment_sum(src, seg, n)
class _Rng:
    def __init__(self, key):
        self._k = key
    def _next(self):
        self._k, sub = jax.random.split(self._k)
        return sub
    def normal(self, shape):
        return jax.random.normal(self._next(), shape, dtype=jnp.bfloat16)
    def randint(self, lo, hi, shape):
        return jax.random.randint(self._next(), shape, lo, hi, dtype=jnp.int32)
    def uniform(self, shape, lo=0.0, hi=1.0):
        return jax.random.uniform(self._next(), shape, jnp.bfloat16, lo, hi)
    def permutation(self, n):
        return jax.random.permutation(self._next(), n)


kernel_name = 'sequential_preLN__sliding_block__glu_gated_glu__prompt'

def setup_inputs():
    _rng = _Rng(jax.random.key(int.from_bytes(__import__("os").urandom(4), "little")))
    _w = (lambda a: (lambda t: t.astype(jnp.bfloat16) if jnp.issubdtype(t.dtype, jnp.floating) else t)(jnp.asarray(a)))
    def _A_setup():
        B, S, D = 1, 2048, 640
        return {
            "x": _w((lambda *s: _rng.normal(s) * 0.05)(B, S, D)),
            "wqkv": _w((lambda *s: _rng.normal(s) * 0.05)(D, 3 * D)),
            "wo": _w((lambda *s: _rng.normal(s) * 0.05)(D, D)),
        }
    _A_in = _A_setup()

    def _B_setup():
        B, S, D, F = 1, 2048, 640, 1728
        return {
            "x": _w((lambda *s: _rng.normal(s) * 0.05)(B, S, D)),
            "w_gate": _w((lambda *s: _rng.normal(s) * 0.05)(D, F)),
            "w_up": _w((lambda *s: _rng.normal(s) * 0.05)(D, F)),
            "w_down": _w((lambda *s: _rng.normal(s) * 0.05)(F, D)),
        }
    _B_in = _B_setup()

    return {
        "A_x": _A_in["x"],
        "A_wqkv": _A_in["wqkv"],
        "A_wo": _A_in["wo"],
        "B_x": _B_in["x"],
        "B_w_gate": _B_in["w_gate"],
        "B_w_up": _B_in["w_up"],
        "B_w_down": _B_in["w_down"],
    }

def reference(A_x, A_wqkv, A_wo, B_x, B_w_gate, B_w_up, B_w_down):
    def _A_ref(x, wqkv, wo):
        B, S, D = x.shape
        H = 32; Dh = D // H; W = 256
        qkv = (lambda x, *d: x.transpose(*d))((x @ wqkv).reshape(B, S, 3, H, Dh), 2, 0, 3, 1, 4)
        q, k, v = qkv[0], qkv[1], qkv[2]
        scores = jnp.einsum("bhqd,bhkd->bhqk", q, k) * (Dh ** -0.5)
        idx = jnp.arange(S)
        mask = (idx[:, None] - idx[None, :] >= 0) & (idx[:, None] - idx[None, :] < W)
        scores = jnp.where(mask[None, None], scores, -1e9)
        p = _softmax(scores, axis=-1)
        o = jnp.einsum("bhqk,bhkd->bhqd", p, v)
        return (lambda x, *d: x.transpose(*d))(o, 0, 2, 1, 3).reshape(B, S, D) @ wo

    def _B_ref(x, w_gate, w_up, w_down):
        g = jnp.einsum("bsd,df->bsf", x, w_gate)
        u = jnp.einsum("bsd,df->bsf", x, w_up)
        h = _sigmoid(g) * u
        return jnp.einsum("bsf,fd->bsd", h, w_down)

    x = A_x
    h = x + _A_ref(_layernorm(x, axis=-1), A_wqkv, A_wo)
    h2 = h + _B_ref(_layernorm(h, axis=-1), B_w_gate, B_w_up, B_w_down)
    return h2
```

```python
import functools, math
import jax, jax.numpy as jnp
from jax import lax
from jax.experimental import pallas as pl
from jax.experimental.pallas import tpu as pltpu

S, D, H, DH, W, F = 2048, 640, 32, 20, 256, 1728
NG = 8
f32 = jnp.float32
bf16 = jnp.bfloat16
u32 = jnp.uint32
NT = (((1,), (1,)), ((), ()))
NH = 4
SB = 32
NBLK = W // SB + 1
FT = F // 128
FR = F - FT * 128
KT = D // 128
NEG = -1e30
T = 256
NB = T // 128
NTILE = S // T
NQ = 2
A0 = NQ + 1


def _ln(x):
    m = jnp.mean(x, axis=-1, keepdims=True)
    xc = x - m
    v = jnp.mean(xc * xc, axis=-1, keepdims=True)
    return xc * lax.rsqrt(v + 1e-5)


def _sigmoid(x):
    return 0.5 * jnp.tanh(0.5 * x) + 0.5


def pull(gen, n):
    last = None
    if gen is None:
        return None
    for _ in range(n):
        v = next(gen, None)
        last = v if v is not None else last
    return last


def mo(v, m):
    return v if isinstance(v, int) else pl.multiple_of(v, m)


def chain(*gens):
    for g in gens:
        yield from g


def make_kernel(LAG, NSLOT, FILL, FILL0, LAG0, GATE, GATE0, TAIL, TAIL0, LNCH, KSPLIT, SMODE):

    def kernel(x_hbm, wqkv_hbm, wo_hbm, wg_hbm, wu_hbm, wd_hbm, o_hbm,
               x_ref, wqkv_ref, wo_ref, wg_ref, wu_ref, wt_ref, wd_ref, sem,
               wvt_ref, k_ref, vt_ref, q_ref, ot_ref, ob_ref, ln1_ref, ln2_ref, h_ref, tmp_ref, o_ref, osem, *pw_refs):
        i = pl.program_id(0)
        k32 = k_ref.bitcast(u32)
        vt32 = vt_ref.bitcast(u32)
        q32 = q_ref.bitcast(u32)
        ob32 = ob_ref.bitcast(u32)
        tmp32 = tmp_ref.bitcast(u32)
        ln32 = ln1_ref.bitcast(u32)
        z1 = i >> 10
        z2 = i >> 11

        def copy(src, dst, n):
            return pltpu.make_async_copy(src, dst, sem.at[n])

        def rows(ref, r0, n):
            return ref.at[pl.ds(r0, n), :]

        def cols(ref, c0, n):
            return ref.at[:, pl.ds(c0, n)]

        def wcopy(c0, n, s):
            return copy(cols(wqkv_hbm, c0, n), cols(wqkv_ref, c0, n), s)

        def xcopy(r0, n, s):
            return copy(rows(x_hbm, r0, n), rows(x_ref, r0, n), s)

        KA = 128 * KSPLIT
        cp_x0 = xcopy(0, T, 0)
        cp_x1 = xcopy(T, T, 1)
        cp_ka = wcopy(D, KA, 2)
        cp_kb = wcopy(D + KA, D - KA, 3)
        cp_v = wcopy(2 * D, D, 4)
        cp_q = wcopy(0, D, 5)
        cp_rest = [copy(wo_hbm, wo_ref, 6),
                   copy(rows(wg_hbm, 0, FT * 128), wg_ref, 7), copy(rows(wu_hbm, 0, FT * 128), wu_ref, 8),
                   copy(rows(wg_hbm, FT * 128, FR), rows(wt_ref, 0, FR), 9),
                   copy(rows(wu_hbm, FT * 128, FR), rows(wt_ref, FR, FR), 10),
                   copy(wd_hbm, wd_ref, 11)]

        lane_h = lax.broadcasted_iota(jnp.int32, (SB // 2, 128), 1)
        rr = lax.broadcasted_iota(jnp.int32, (SB, 128), 0)
        ll = lax.broadcasted_iota(jnp.int32, (SB, 128), 1)
        tri = rr <= (ll & (SB - 1))
        r8 = lax.broadcasted_iota(jnp.int32, (8, 128), 0)
        zero_blk = jnp.zeros((SB // 2, 128), u32)
        mk1 = (lane_h & SB) != 0
        mk2 = (lane_h & (2 * SB)) != 0
        never = r8 < (i >> 10)

        pending = []

        def ln1_gen(base, n, ch, d0=0):
            for r in range(d0, d0 + n, ch):
                y = _ln(x_ref[pl.ds(mo(base + r - d0, 16), ch), :].astype(f32))
                tok = None
                for k in range(KT):
                    ln1_ref[k, r:r + ch, :] = y[:, k * 128:(k + 1) * 128].astype(bf16)
                    for s in range(r // 2, (r + ch) // 2, 8):
                        w = ln32[k, s:s + 8, :]
                        tok = w if tok is None else tok | w
                pending.append(tok)
                yield

        def ln1_load(half):
            return [ln32[k, half * (T // 2):(half + 1) * (T // 2), :] for k in range(KT)]

        def gated(u):
            if pending:
                u = jnp.concatenate([jnp.where(never, pending.pop(), u[:8]), u[8:]], axis=0)
            return pltpu.bitcast(u, bf16)

        def weave(gen, side, every, start=0):
            for n, v in enumerate(gen):
                yield v
                if n >= start and (n - start) % every == every - 1:
                    next(side, None)
            for _ in side:
                pass
            pending.clear()

        def proj_gen(ln1, col0, store):
            laneT = lax.broadcasted_iota(jnp.int32, (T, 128), 1)
            tiles = []
            done = 0
            for n in range(KT):
                acc = None
                for k in range(KT):
                    p = jnp.dot(gated(ln1[k]),
                                wqkv_ref[k * 128:(k + 1) * 128, col0 + n * 128:col0 + (n + 1) * 128],
                                preferred_element_type=f32)
                    acc = p if acc is None else p + acc
                    if k == KT - 1:
                        tiles.append(acc)
                        while done < NG and (80 * done + 79) // 128 <= n:
                            lo = 80 * done
                            ta, tb = lo // 128, (lo + 79) // 128
                            a = tiles[ta]
                            if tb != ta:
                                a = jnp.where(laneT >= lo % 128, a, tiles[tb])
                            store(done, a)
                            done += 1
                    yield acc

        def k_gen(ln1, tile):
            def store(g, a):
                k_ref[g, pl.ds(mo(tile * T, T), T), :] = a.astype(bf16)
            return proj_gen(ln1, D, store)

        def q_gen(ln1, tile):
            qscale = DH ** -0.5 * math.log2(math.e)

            def store(g, a):
                q_ref[g, pl.ds(mo(tile * T, T), T), :] = (a * qscale).astype(bf16)
            return proj_gen(ln1, 0, store)

        def v_gen(ln1, tile):
            blk = tile * NB
            r32 = lax.broadcasted_iota(jnp.int32, (32, 128), 0)
            for b in range(NB):
                for hf in range(2):
                    acc = None
                    for k in range(KT):
                        p = lax.dot_general(wvt_ref[hf * 320:(hf + 1) * 320, k * 128:(k + 1) * 128],
                                            gated(ln1[k][b * 64:(b + 1) * 64]), NT,
                                            preferred_element_type=f32)
                        acc = p if acc is None else p + acc
                        if k == KT - 1:
                            for h in range(hf * 16, hf * 16 + 16):
                                a = (5 * h) // 4 - hf * 20
                                o = 4 * (h % 4)
                                vh = jnp.where((r32 >= o) & (r32 < o + DH), acc[16 * a:16 * a + 32, :], 1.0)
                                vt_ref[blk + b, h * 32:(h + 1) * 32, :] = vh.astype(bf16)
                        yield acc

        def nskip(first, b, c):
            return max(0, (W - b * 128 - c * SB) // SB) if first else 0

        def stage_qk(first, hbase, b, g):
            res = {}
            for c in [(cc + (g if first else 0)) % NH for cc in range(NH)]:
                hq = hbase + (b * 128 + c * SB) // 2
                if not first:
                    hq = pl.multiple_of(hq, SB // 2)
                qs = q32[g, pl.ds(hq, SB // 2), :]
                wrows = []
                for j in range(NH):
                    hh = 4 * g + (j ^ c)
                    mk = ((lane_h - (20 * hh) % 128) & 127) < DH
                    wrows.append(jnp.where(mk, qs, zero_blk))
                wc = pltpu.bitcast(jnp.concatenate(wrows, axis=0), bf16)
                ns = nskip(first, b, c)
                parts = [k32[g, pl.ds(hq, SB // 2), :]]
                if ns < 8:
                    parts.append(k32[g, pl.ds(hq - (W - ns * SB) // 2, (W - ns * SB) // 2), :])
                kw = jnp.concatenate(parts, axis=0) if len(parts) > 1 else parts[0]
                s = lax.dot_general(pltpu.bitcast(kw, bf16), wc, NT, preferred_element_type=f32)
                if ns == 0:
                    mrg = jnp.where(tri, s[:SB], s[SB:2 * SB])
                    sm = jnp.concatenate([mrg, s[2 * SB:]], axis=0)
                else:
                    mrg = jnp.where(tri, s[:SB], NEG)
                    sm = jnp.concatenate([mrg, s[SB:]], axis=0) if ns < 8 else mrg
                m = jnp.max(jnp.max(sm.reshape(sm.shape[0] // 8, 8, 128), axis=0), axis=0, keepdims=True)
                res[c] = (sm, m)
            return res

        def sel(mk, hi_, lo_):
            if lo_ is None and hi_ is None:
                return None
            return jnp.where(mk, zero_blk if hi_ is None else hi_, zero_blk if lo_ is None else lo_)

        def pack(n, v):
            tmp_ref[n] = v.astype(bf16)
            return tmp32[n]

        def stage_exp(first, b, slot, sres, toks, gate):
            pm = [jnp.exp2(sres[c][0][:SB] - sres[c][1]) for c in range(NH)]
            rho0 = max(0, 8 - 4 * b) if first else 0
            for rho in range(rho0, 12):
                cur = []
                for c in range(NH):
                    ns = nskip(first, b, c)
                    sm, m = sres[c]
                    j = rho - c
                    n = rho * NH + c
                    if j < ns or j >= NBLK:
                        cur.append(None)
                    elif j == NBLK - 1:
                        cur.append(pack(n, jnp.where(tri, pm[c], 0.0) if ns == 0 else pm[c]))
                    elif j == 0:
                        cur.append(pack(n, jnp.where(tri, 0.0, pm[c])))
                    else:
                        r0 = (j - ns + (1 if ns else 0)) * SB
                        if toks:
                            ntok = len(toks) * 32
                            pos = gate[0] + ((rho - rho0) * (ntok - gate[0] - gate[1])) // (12 - rho0)
                            tok = toks[pos // 32][(pos % 32) * 8:(pos % 32) * 8 + 8]
                            mg = jnp.where(never, tok, jnp.broadcast_to(m, (8, 128)))
                            d = (sm[r0:r0 + SB].reshape(4, 8, 128) - mg[None]).reshape(SB, 128)
                        else:
                            d = sm[r0:r0 + SB] - m
                        cur.append(pack(n, jnp.exp2(d)))
                cur = [sel(mk1, cur[e ^ 1], cur[e]) for e in range(NH)]
                cur = [sel(mk2, cur[e ^ 2], cur[e]) for e in range(NH)]
                for e in range(NH):
                    pw_refs[slot][z1, e, rho * 16:(rho + 1) * 16, :] = cur[e]

        def stage_pv(first, blk, b, g, slot, after):
            vb = blk + b - 2
            res = [None] * NH
            for t in range(3):
                if not (first and b + t < 2):
                    for e in range(NH):
                        h = 4 * g + e
                        pe = pltpu.bitcast(pw_refs[slot][z2, e, t * 64:(t + 1) * 64, :], bf16)
                        vw = pltpu.bitcast(vt32[vb + t, h * 16:(h + 1) * 16, :], bf16)
                        r = jnp.dot(vw, pe, preferred_element_type=f32)
                        res[e] = r if res[e] is None else r + res[e]
                after(t)
            outs = []
            for e in range(NH):
                r = res[e]
                if e < 2:
                    inv = 1.0 / r[24:32]
                    outs.append([r[8 * t:8 * t + 8] * inv for t in range(3)])
                else:
                    inv = 1.0 / r[0:8]
                    outs.append([r[8 * t:8 * t + 8] * inv for t in range(1, 4)])
            lo4 = r8 < 4
            rws = [outs[0][0], outs[0][1], jnp.where(lo4, outs[0][2], outs[1][0]), outs[1][1], outs[1][2],
                   outs[2][0], outs[2][1], jnp.where(lo4, outs[2][2], outs[3][0]), outs[3][1], outs[3][2]]
            ot_ref[g * 80:(g + 1) * 80, b * 128:(b + 1) * 128] = jnp.concatenate(rws, axis=0)

        def attention(first, tile, gen, lag, fillf, gate):
            hbase = tile * (T // 2)
            blk = tile * NB
            units = [(b, g) for b in range(NB) for g in range(NG)]
            pend = []
            for u in range(len(units) + lag):
                if u < len(units):
                    pend.append(stage_qk(first, hbase, *units[u]))
                toks = []
                fill = fillf(u)

                def after(t):
                    v = pull(gen, fill[t])
                    if v is not None and len(toks) < gate[2]:
                        toks.append(v)
                if u >= lag:
                    stage_pv(first, blk, *units[u - lag], (u - lag) % NSLOT, after)
                else:
                    for t in range(3):
                        after(t)
                if u < len(units):
                    stage_exp(first, units[u][0], u % NSLOT, pend[u], toks, gate)

        def out_proj(base, nsplit, parts=2):
            o_t = ot_ref[...].T
            for t in range(KT):
                ob_ref[t] = o_t[:, t * 128:(t + 1) * 128].astype(bf16)
            cols = []
            for t in range(KT):
                e_lane = ((lane_h + t * 128) // DH) % NH
                blks = [ob32[t, r * 16:(r + 1) * 16, :] for r in range(T // SB)]
                for bit in (1, 2):
                    mk = (e_lane & bit) != 0
                    blks = [jnp.where(mk, blks[r ^ bit], blks[r]) for r in range(T // SB)]
                cols.append(pltpu.bitcast(jnp.concatenate(blks, axis=0), bf16))
            outs = []
            cnt = 0
            for n in range(KT):
                acc = x_ref[pl.ds(base, T), n * 128:(n + 1) * 128].astype(f32)
                for k in range(KT):
                    w = wo_ref[k * 128:(k + 1) * 128, n * 128:(n + 1) * 128]
                    if cnt < nsplit:
                        acc = jnp.concatenate(
                            [jnp.dot(cols[k][hf * (T // parts):(hf + 1) * (T // parts)], w, preferred_element_type=f32)
                             + acc[hf * (T // parts):(hf + 1) * (T // parts)] for hf in range(parts)], axis=0)
                    else:
                        acc = jnp.dot(cols[k], w, preferred_element_type=f32) + acc
                    cnt += 1
                outs.append(acc)
            return jnp.concatenate(outs, axis=1)

        def save_h(hres):
            h_ref[...] = hres
            ln2_ref[...] = _ln(hres).astype(bf16)

        def ffn_gen(tile, done=None):
            ln2 = [ln2_ref[:, k * 128:(k + 1) * 128] for k in range(KT)]
            acts = []

            def proj(w_ref, r0):
                acc = None
                for k in range(KT):
                    p = lax.dot_general(ln2[k], w_ref[r0:r0 + 128, k * 128:(k + 1) * 128], NT, preferred_element_type=f32)
                    acc = p if acc is None else p + acc
                    if k == KT - 1:
                        res.append(acc)
                    yield acc

            for j in range(FT):
                res = []
                yield from proj(wg_ref, j * 128)
                yield from proj(wu_ref, j * 128)
                acts.append((_sigmoid(res[0]) * res[1]).astype(bf16))
            res = []
            yield from proj(wt_ref, 0)
            acts.append((_sigmoid(res[0]) * pltpu.roll(res[0], FR, 1))[:, :FR].astype(bf16))
            for n in range(KT):
                acc = h_ref[:, n * 128:(n + 1) * 128]
                for j in range(FT + 1):
                    r1 = min(F, (j + 1) * 128)
                    acc = jnp.dot(acts[j], wd_ref[j * 128:r1, n * 128:(n + 1) * 128], preferred_element_type=f32) + acc
                    if j == FT:
                        o_ref[pl.ds(mo(tile * T, T), T), n * 128:(n + 1) * 128] = acc.astype(o_ref.dtype)
                        if done is not None:
                            done(n)
                    yield acc

        def ocopy(tile):
            return pltpu.make_async_copy(rows(o_ref, mo(tile * T, T), T), rows(o_hbm, mo(tile * T, T), T), osem.at[tile])

        def ocopy_last(n):
            sl = (pl.ds(S - T, T), pl.ds(n * 128, 128))
            return pltpu.make_async_copy(o_ref.at[sl], o_hbm.at[sl], osem.at[NTILE - 1 + n])

        @pl.when(i == 0)
        def _start():
            cp_xs = [xcopy(2 * T * (j + 1), 2 * T, 12 + j) for j in range(3)]
            for cp in [cp_x0, cp_x1, cp_ka, cp_kb, cp_q, cp_v] + cp_xs + cp_rest:
                cp.start()
            cp_x0.wait()
            pull(ln1_gen(0, T, T), 1)
            cp_x1.wait()
            pull(ln1_gen(T, T, T, T), 1)
            pending.clear()
            la, lb = ln1_load(0), ln1_load(1)
            ga, gb = k_gen(la, 0), k_gen(lb, 1)
            cp_ka.wait()
            pull(ga, KSPLIT * KT)
            pull(gb, KSPLIT * KT)
            cp_kb.wait()
            if SMODE == 0:
                pull(chain(ga, gb), 100)
                cp_q.wait()
                cp_v.wait()
                wvt_ref[...] = wqkv_ref[:, 2 * D:].T
                pull(chain(q_gen(la, 0), q_gen(lb, 1)), 100)
                cp_xs[0].wait()
                pull(weave(chain(v_gen(la, 0), v_gen(lb, 1)), ln1_gen(2 * T, 2 * T, 32), 2, 4), 100)
            else:
                cp_q.wait()
                pull(chain(ga, gb, q_gen(la, 0)), 100)
                cp_v.wait()
                cp_xs[0].wait()
                wvt_ref[...] = wqkv_ref[:, 2 * D:].T
                pull(weave(chain(q_gen(lb, 1), v_gen(la, 0), v_gen(lb, 1)), ln1_gen(2 * T, 2 * T, 32), 2, 28), 100)

        @pl.when((i > 0) & (i < A0))
        def _qkv():
            t0 = 2 * i
            nxt = pl.multiple_of((t0 + 2) * T, T)
            copy(rows(x_hbm, nxt, 2 * T), rows(x_ref, nxt, 2 * T), 12 + i).wait()
            la, lb = ln1_load(0), ln1_load(1)
            pull(weave(chain(k_gen(la, t0), k_gen(lb, t0 + 1), q_gen(la, t0), q_gen(lb, t0 + 1), v_gen(la, t0), v_gen(lb, t0 + 1)),
                       ln1_gen(nxt, 2 * T, LNCH[0]), LNCH[1], LNCH[2]), 1000)

        @pl.when(i == A0)
        def _first():
            for cp in cp_rest:
                cp.wait()
            t0 = NTILE - 2
            la, lb = ln1_load(0), ln1_load(1)
            gen = chain(k_gen(la, t0), k_gen(lb, t0 + 1), q_gen(la, t0), q_gen(lb, t0 + 1), v_gen(la, t0), v_gen(lb, t0 + 1))
            attention(True, 0, gen, LAG0, lambda u: FILL0[0] if u < FILL0[1] else FILL0[2], GATE0)
            pull(gen, TAIL0[0])
            hres = out_proj(0, TAIL0[1], 4)
            pull(gen, 1000)
            save_h(hres)

        @pl.when((i > A0) & (i < A0 + NTILE))
        def _main():
            tile = i - A0
            gen = ffn_gen(tile - 1)
            attention(False, tile, gen, LAG, lambda u: FILL[0] if u < FILL[1] else FILL[2], GATE)
            pull(gen, TAIL[0])
            hres = out_proj(pl.multiple_of(tile * T, T), TAIL[1])
            pull(gen, 1000)
            save_h(hres)
            ocopy(tile - 1).start()

        @pl.when(i == A0 + NTILE)
        def _last():
            pull(ffn_gen(NTILE - 1, lambda n: ocopy_last(n).start()), 1000)
            for t in range(NTILE - 1):
                ocopy(t).wait()
            for n in range(KT):
                ocopy_last(n).wait()

    return kernel


_PARAMS = dict(LAG=1, NSLOT=3, FILL=((4, 4, 4), 10, (4, 4, 0)), FILL0=((0, 0, 4), 8, (0, 4, 4)), LAG0=1, GATE=(0, 8, 2), GATE0=(0, 8, 2),
          TAIL=(12, 2), TAIL0=(12, 1), LNCH=(32, 6, 32), KSPLIT=2, SMODE=0)


@jax.jit
def pallas_sequential_preLN__sliding_block__glu_gated_glu__prompt_kernel(A_x, A_wqkv, A_wo, B_x, B_w_gate, B_w_up, B_w_down):
    x = A_x.reshape(S, D)
    anyspec = pl.BlockSpec(memory_space=pl.ANY)
    out = pl.pallas_call(
        make_kernel(**_PARAMS),
        grid=(A0 + NTILE + 1,),
        in_specs=[anyspec] * 6,
        out_specs=anyspec,
        out_shape=jax.ShapeDtypeStruct((S, D), bf16),
        scratch_shapes=[pltpu.VMEM((S, D), bf16),
                        pltpu.VMEM((D, 3 * D), bf16),
                        pltpu.VMEM((D, D), bf16),
                        pltpu.VMEM((FT * 128, D), bf16),
                        pltpu.VMEM((FT * 128, D), bf16),
                        pltpu.VMEM((2 * FR, D), bf16),
                        pltpu.VMEM((F, D), bf16),
                        pltpu.SemaphoreType.DMA((15,)),
                        pltpu.VMEM((D, D), bf16),
                        pltpu.VMEM((NG, S, 128), bf16),
                        pltpu.VMEM((S // 128, H * 32, 128), bf16),
                        pltpu.VMEM((NG, S, 128), bf16),
                        pltpu.VMEM((D, T), f32),
                        pltpu.VMEM((KT, T, 128), bf16),
                        pltpu.VMEM((KT, 2 * T, 128), bf16),
                        pltpu.VMEM((T, D), bf16),
                        pltpu.VMEM((T, D), f32),
                        pltpu.VMEM((48, SB, 128), bf16),
                        pltpu.VMEM((S, D), bf16),
                        pltpu.SemaphoreType.DMA((NTILE - 1 + KT,))]
        + [pltpu.VMEM((1, NH, 192, 128), u32)] * _PARAMS["NSLOT"],
        compiler_params=pltpu.CompilerParams(dimension_semantics=("arbitrary",),
                                             vmem_limit_bytes=100 * 1024 * 1024),
    )(x, A_wqkv, A_wo, B_w_gate.T, B_w_up.T, B_w_down)
    return out.reshape(1, S, D)
```

```python
import math

import jax
import jax.numpy as jnp
from jax import lax
from jax.experimental import pallas as pl
from jax.experimental.pallas import tpu as pltpu

S, D, H, DH, W, F = 2048, 640, 32, 20, 256, 1728
f32 = jnp.float32
bf16 = jnp.bfloat16
u32 = jnp.uint32
NT = (((1,), (1,)), ((), ()))
NG = 8
NH = 4
SB = 32
NBLK = W // SB + 1
FT = F // 128
FR = F - FT * 128
KT = D // 128
NEG = -1e30
T = 256
NB = T // 128
NTILE = S // T

LAG, FILL, GATE, TAIL, PRE = 1, ((4, 4, 0), 7, (4, 4, 4)), (0, 4, 2), (4, (2, 2, 4)), 3
LAG0, FILL0, GATE0, TAIL0, PRE0 = 2, ((0, 0, 4), 10, (0, 4, 4)), (0, 0, 2), (4, (2, 2)), 1
KSPLIT, REGIONS = 2, (20, 16, 52, 100)


def _ln(x):
    m = jnp.mean(x, axis=-1, keepdims=True)
    xc = x - m
    v = jnp.mean(xc * xc, axis=-1, keepdims=True)
    return xc * lax.rsqrt(v + 1e-5)


def _sigmoid(x):
    return 0.5 * jnp.tanh(0.5 * x) + 0.5


def _pack(v):
    return pltpu.bitcast(v.astype(bf16), u32)


def _unpack(u):
    return pltpu.bitcast(u, bf16)


def _pull(gen, n):
    last = None
    for _ in range(n):
        v = next(gen, None)
        last = v if v is not None else last
    return last


def _mo(v, m):
    return v if isinstance(v, int) else pl.multiple_of(v, m)


def _chain(*gens):
    for g in gens:
        yield from g


def _take(g, n):
    for _ in range(n):
        yield next(g)


def _kernel(x_hbm, wqkv_hbm, wo_hbm, wg_hbm, wu_hbm, wd_hbm, o_hbm,
            x_ref, wqkv_ref, wo_ref, wg_ref, wu_ref, wt_ref, wd_ref, sem,
            wvt_ref, k_ref, vt_ref, q_ref, ot_ref, ln1_ref, ln2_ref, h_ref, o_ref, osem):
    i = pl.program_id(0)
    zero = i >> 10

    def copy(src, dst, n):
        return pltpu.make_async_copy(src, dst, sem.at[n])

    def rows(ref, r0, n):
        return ref.at[pl.ds(r0, n), :]

    def cols(ref, c0, n):
        return ref.at[:, pl.ds(c0, n)]

    def wcopy(c0, n, s):
        return copy(cols(wqkv_hbm, c0, n), cols(wqkv_ref, c0, n), s)

    def xcopy(r0, n, s):
        return copy(rows(x_hbm, r0, n), rows(x_ref, r0, n), s)

    lane_h = lax.broadcasted_iota(jnp.int32, (SB // 2, 128), 1)
    rr = lax.broadcasted_iota(jnp.int32, (SB, 128), 0)
    ll = lax.broadcasted_iota(jnp.int32, (SB, 128), 1)
    tri = rr <= (ll & (SB - 1))
    r8 = lax.broadcasted_iota(jnp.int32, (8, 128), 0)
    zero_u = jnp.zeros((SB // 2, 128), u32)
    never8 = r8 < zero
    never32 = rr < zero
    mk1 = (lane_h & SB) != 0
    mk2 = (lane_h & (2 * SB)) != 0

    def ln1_chunk(r, ch, tok=None):
        x = x_ref[r:r + ch, :].astype(f32)
        if tok is not None:
            x = jnp.concatenate([jnp.where(never32, tok[:ch], x[:, :128]), x[:, 128:]], axis=1)
        y = _ln(x)
        for k in range(KT):
            ln1_ref[k, r:r + ch, :] = y[:, k * 128:(k + 1) * 128].astype(bf16)

    def ln1_tile(tile, k, r0=0, n=T):
        return ln1_ref[k, pl.ds(_mo(tile * T + r0, 128), n), :]

    def weave(gen, n, r0, nrows, every, free):
        todo = list(range(r0, r0 + nrows, SB))
        for _ in range(free):
            ln1_chunk(todo.pop(0), SB)
        for j in range(n):
            acc = next(gen)
            if todo and j % every == 0:
                ln1_chunk(todo.pop(0), SB, acc)
        assert not todo

    def proj_gen(tile, col0, store):
        lane_t = lax.broadcasted_iota(jnp.int32, (T, 128), 1)
        tiles = []
        done = 0
        for n in range(KT):
            acc = None
            for k in range(KT):
                p = jnp.dot(ln1_tile(tile, k),
                            wqkv_ref[k * 128:(k + 1) * 128, col0 + n * 128:col0 + (n + 1) * 128],
                            preferred_element_type=f32)
                acc = p if acc is None else p + acc
                if k == KT - 1:
                    tiles.append(acc)
                    while done < NG and (80 * done + 79) // 128 <= n:
                        lo = 80 * done
                        ta, tb = lo // 128, (lo + 79) // 128
                        a = tiles[ta]
                        if tb != ta:
                            a = jnp.where(lane_t >= lo % 128, a, tiles[tb])
                        store(done, a)
                        done += 1
                yield acc

    def k_gen(tile):
        def store(g, a):
            k_ref[g, tile * (T // 2):(tile + 1) * (T // 2), :] = _pack(a)
        return proj_gen(tile, D, store)

    def q_gen(tile):
        qscale = DH ** -0.5 * math.log2(math.e)

        def store(g, a):
            q_ref[g] = _pack(a * qscale)
        return proj_gen(tile, 0, store)

    def v_gen(tile):
        for b in range(NB):
            for hf in range(2):
                acc = None
                for k in range(KT):
                    p = lax.dot_general(wvt_ref[hf * 320:(hf + 1) * 320, k * 128:(k + 1) * 128],
                                        ln1_tile(tile, k, b * 128, 128), NT, preferred_element_type=f32)
                    acc = p if acc is None else p + acc
                    if k == KT - 1:
                        for h in range(hf * 16, hf * 16 + 16):
                            a = (5 * h) // 4 - hf * 20
                            o = 4 * (h % 4)
                            vh = jnp.where((rr >= o) & (rr < o + DH), acc[16 * a:16 * a + 32, :], 1.0)
                            vt_ref[tile * NB + b, h * 16:(h + 1) * 16, :] = _pack(vh)
                    yield acc

    def nskip(first, b, c):
        return max(0, (W - b * 128 - c * SB) // SB) if first else 0

    def stage_qk(first, hbase, b, g):
        res = {}
        for c in [(cc + (g if first else 0)) % NH for cc in range(NH)]:
            r0 = (b * 128 + c * SB) // 2
            q0 = _mo(hbase + r0, SB // 2)
            qs = q_ref[g, r0:r0 + SB // 2, :]
            wrows = []
            for j in range(NH):
                hh = 4 * g + (j ^ c)
                mk = ((lane_h - (20 * hh) % 128) & 127) < DH
                wrows.append(jnp.where(mk, qs, zero_u))
            wc = _unpack(jnp.concatenate(wrows, axis=0))
            ns = nskip(first, b, c)
            parts = [k_ref[g, pl.ds(q0, SB // 2), :]]
            if ns < 8:
                parts.append(k_ref[g, pl.ds(q0 - (W - ns * SB) // 2, (W - ns * SB) // 2), :])
            kw = jnp.concatenate(parts, axis=0) if len(parts) > 1 else parts[0]
            s = lax.dot_general(_unpack(kw), wc, NT, preferred_element_type=f32)
            if ns == 0:
                mrg = jnp.where(tri, s[:SB], s[SB:2 * SB])
                sm = jnp.concatenate([mrg, s[2 * SB:]], axis=0)
            else:
                mrg = jnp.where(tri, s[:SB], NEG)
                sm = jnp.concatenate([mrg, s[SB:]], axis=0) if ns < 8 else mrg
            m = jnp.max(jnp.max(sm.reshape(sm.shape[0] // 8, 8, 128), axis=0), axis=0, keepdims=True)
            res[c] = (sm, m)
        return res

    def sel(mk, hi, lo):
        if lo is None and hi is None:
            return None
        return jnp.where(mk, zero_u if hi is None else hi, zero_u if lo is None else lo)

    def stage_exp(first, b, sres, toks, gate):
        pm = [jnp.exp2(sres[c][0][:SB] - sres[c][1]) for c in range(NH)]
        rho0 = max(0, 8 - 4 * b) if first else 0
        pw = [{} for _ in range(NH)]
        blks = [[] for _ in range(NH)]
        for rho in range(rho0, 12):
            cur = []
            for c in range(NH):
                ns = nskip(first, b, c)
                sm, m = sres[c]
                j = rho - c
                if j < ns or j >= NBLK:
                    cur.append(None)
                elif j == NBLK - 1:
                    cur.append(_pack(jnp.where(tri, pm[c], 0.0) if ns == 0 else pm[c]))
                elif j == 0:
                    cur.append(_pack(jnp.where(tri, 0.0, pm[c])))
                else:
                    r0 = (j - ns + (1 if ns else 0)) * SB
                    if toks:
                        ntok = len(toks) * 32
                        pos = gate[0] + ((rho - rho0) * (ntok - gate[0] - gate[1])) // (12 - rho0)
                        tok = toks[pos // 32][(pos % 32) * 8:(pos % 32) * 8 + 8]
                        mg = jnp.where(never8, tok, jnp.broadcast_to(m, (8, 128)))
                        d = (sm[r0:r0 + SB].reshape(4, 8, 128) - mg[None]).reshape(SB, 128)
                    else:
                        d = sm[r0:r0 + SB] - m
                    cur.append(_pack(jnp.exp2(d)))
            cur = [sel(mk1, cur[e ^ 1], cur[e]) for e in range(NH)]
            cur = [sel(mk2, cur[e ^ 2], cur[e]) for e in range(NH)]
            for e in range(NH):
                blks[e].append(cur[e])
                if rho % 4 == 3:
                    pw[e][rho // 4] = _unpack(jnp.concatenate(blks[e], axis=0))
                    blks[e] = []
        return pw

    def stage_pv(blk, b, g, pw, after):
        vb = blk + b - 2
        res = [None] * NH
        for t in range(3):
            if t in pw[0]:
                for e in range(NH):
                    h = 4 * g + e
                    r = jnp.dot(_unpack(vt_ref[vb + t, h * 16:(h + 1) * 16, :]), pw[e][t],
                                preferred_element_type=f32)
                    res[e] = r if res[e] is None else r + res[e]
            after(t)
        outs = []
        for e in range(NH):
            r = res[e]
            if e < 2:
                inv = 1.0 / r[24:32]
                outs.append([r[8 * t:8 * t + 8] * inv for t in range(3)])
            else:
                inv = 1.0 / r[0:8]
                outs.append([r[8 * t:8 * t + 8] * inv for t in range(1, 4)])
        lo4 = r8 < 4
        rws = [outs[0][0], outs[0][1], jnp.where(lo4, outs[0][2], outs[1][0]), outs[1][1], outs[1][2],
               outs[2][0], outs[2][1], jnp.where(lo4, outs[2][2], outs[3][0]), outs[3][1], outs[3][2]]
        ot_ref[g * 80:(g + 1) * 80, b * 128:(b + 1) * 128] = jnp.concatenate(rws, axis=0)

    def attention(first, tile, gen, lag, fills, gate):
        units = [(b, g) for b in range(NB) for g in range(NG)]
        pws = []
        for u in range(len(units) + lag):
            if u < len(units):
                sres = stage_qk(first, tile * (T // 2), *units[u])
            toks = []
            fill = fills[0] if u < fills[1] else fills[2]

            def after(t):
                v = _pull(gen, fill[t])
                if v is not None and len(toks) < gate[2]:
                    toks.append(v)
            if u >= lag:
                stage_pv(tile * NB, *units[u - lag], pws[u - lag], after)
            else:
                for t in range(3):
                    after(t)
            if u < len(units):
                pws.append(stage_exp(first, units[u][0], sres, toks, gate))

    def out_proj(base, split):
        o_t = ot_ref[...].T
        lhs = []
        for t in range(KT):
            e_lane = ((lane_h + t * 128) // DH) % NH
            ob = _pack(o_t[:, t * 128:(t + 1) * 128])
            blks = [ob[r * 16:(r + 1) * 16, :] for r in range(T // SB)]
            for bit in (1, 2):
                mk = (e_lane & bit) != 0
                blks = [jnp.where(mk, blks[r ^ bit], blks[r]) for r in range(T // SB)]
            lhs.append(_unpack(jnp.concatenate(blks, axis=0)))
        outs = []
        cnt = 0
        for n in range(KT):
            acc = x_ref[pl.ds(base, T), n * 128:(n + 1) * 128].astype(f32)
            for k in range(KT):
                w = wo_ref[k * 128:(k + 1) * 128, n * 128:(n + 1) * 128]
                if cnt < len(split):
                    m = T // split[cnt]
                    acc = jnp.concatenate(
                        [jnp.dot(lhs[k][r:r + m], w, preferred_element_type=f32) + acc[r:r + m]
                         for r in range(0, T, m)], axis=0)
                else:
                    acc = jnp.dot(lhs[k], w, preferred_element_type=f32) + acc
                cnt += 1
            outs.append(acc)
        return jnp.concatenate(outs, axis=1)

    def save_h(hres):
        h_ref[...] = hres
        ln2_ref[...] = _ln(hres).astype(bf16)

    def ffn_gen(tile, done=None):
        ln2 = [ln2_ref[:, k * 128:(k + 1) * 128] for k in range(KT)]
        acts = []

        def proj(w_ref, r0):
            acc = None
            for k in range(KT):
                p = lax.dot_general(ln2[k], w_ref[r0:r0 + 128, k * 128:(k + 1) * 128], NT,
                                    preferred_element_type=f32)
                acc = p if acc is None else p + acc
                if k == KT - 1:
                    res.append(acc)
                yield acc

        for j in range(FT):
            res = []
            yield from proj(wg_ref, j * 128)
            yield from proj(wu_ref, j * 128)
            acts.append((_sigmoid(res[0]) * res[1]).astype(bf16))
        res = []
        yield from proj(wt_ref, 0)
        acts.append((_sigmoid(res[0]) * pltpu.roll(res[0], FR, 1))[:, :FR].astype(bf16))
        for n in range(KT):
            acc = h_ref[:, n * 128:(n + 1) * 128]
            for j in range(FT + 1):
                r1 = min(F, (j + 1) * 128)
                acc = jnp.dot(acts[j], wd_ref[j * 128:r1, n * 128:(n + 1) * 128],
                              preferred_element_type=f32) + acc
                if j == FT:
                    o_ref[pl.ds(_mo(tile * T, T), T), n * 128:(n + 1) * 128] = acc.astype(o_ref.dtype)
                    if done is not None:
                        done(n)
                yield acc

    def ocopy(tile):
        r0 = _mo(tile * T, T)
        return pltpu.make_async_copy(rows(o_ref, r0, T), rows(o_hbm, r0, T), osem.at[tile])

    def ocopy_last(n):
        sl = (pl.ds(S - T, T), pl.ds(n * 128, 128))
        return pltpu.make_async_copy(o_ref.at[sl], o_hbm.at[sl], osem.at[NTILE - 1 + n])

    @pl.when(i == 0)
    def _start():
        ka = 128 * KSPLIT
        cp_x0, cp_x1 = xcopy(0, T, 0), xcopy(T, T, 1)
        cp_ka, cp_kb = wcopy(D, ka, 2), wcopy(D + ka, D - ka, 3)
        cp_v, cp_q = wcopy(2 * D, D, 4), wcopy(0, D, 5)
        cp_o = copy(wo_hbm, wo_ref, 6)
        cp_ffn = [copy(rows(wg_hbm, 0, FT * 128), wg_ref, 7), copy(rows(wu_hbm, 0, FT * 128), wu_ref, 8),
                  copy(rows(wg_hbm, FT * 128, FR), rows(wt_ref, 0, FR), 9),
                  copy(rows(wu_hbm, FT * 128, FR), rows(wt_ref, FR, FR), 10),
                  copy(wd_hbm, wd_ref, 11)]
        cp_xs = [xcopy(2 * T * (j + 1), 2 * T, 12 + j) for j in range(3)]
        for cp in [cp_x0, cp_x1, cp_ka, cp_kb, cp_xs[0], cp_v, cp_xs[1], cp_q, cp_xs[2], cp_o] + cp_ffn:
            cp.start()
        cp_x0.wait()
        ln1_chunk(0, T)
        cp_x1.wait()
        ln1_chunk(T, T)
        g0, g1, g6 = k_gen(0), k_gen(1), k_gen(6)
        gen = _chain(_take(g0, KSPLIT * KT), _take(g1, KSPLIT * KT), g0, g1, k_gen(2), k_gen(3),
                     v_gen(0), v_gen(1), k_gen(4), k_gen(5), v_gen(2), v_gen(3), q_gen(0),
                     _take(g6, 1), v_gen(4), v_gen(5), v_gen(6), v_gen(7), g6, k_gen(7))
        n1, n2, n3, n4 = REGIONS
        cp_ka.wait()
        _pull(gen, n1)
        cp_kb.wait()
        _pull(gen, n2)
        cp_xs[0].wait()
        left = 50 - n1 - n2
        weave(gen, left, 2 * T, T, 2, 2)
        weave(gen, 25, 3 * T, T, 2, 0)
        _pull(gen, n3 - left - 25)
        cp_v.wait()
        cp_xs[1].wait()
        wvt_ref[...] = wqkv_ref[:, 2 * D:].T
        left = 100 - n1 - n2 - n3
        _pull(gen, left)
        weave(gen, 40, 4 * T, 2 * T, 2, 0)
        _pull(gen, n4 - left - 40)
        cp_q.wait()
        cp_xs[2].wait()
        cp_o.wait()
        left = 230 - n1 - n2 - n3 - n4
        weave(gen, left + 25, 6 * T, 2 * T, 3, 0)
        _pull(gen, PRE0)
        attention(True, 0, gen, LAG0, FILL0, GATE0)
        _pull(gen, TAIL0[0])
        hres = out_proj(0, TAIL0[1])
        _pull(gen, 1000)
        save_h(hres)
        for cp in cp_ffn:
            cp.wait()

    @pl.when((i > 0) & (i < NTILE))
    def _main():
        _pull(q_gen(i), 100)
        gen = ffn_gen(i - 1)
        _pull(gen, PRE)
        attention(False, i, gen, LAG, FILL, GATE)
        _pull(gen, TAIL[0])
        hres = out_proj(pl.multiple_of(i * T, T), TAIL[1])
        _pull(gen, 1000)
        save_h(hres)
        ocopy(i - 1).start()

    @pl.when(i == NTILE)
    def _last():
        _pull(ffn_gen(NTILE - 1, lambda n: ocopy_last(n).start()), 1000)
        for t in range(NTILE - 1):
            ocopy(t).wait()
        for n in range(KT):
            ocopy_last(n).wait()


@jax.jit
def pallas_sequential_preLN__sliding_block__glu_gated_glu__prompt_kernel(
    A_x: jax.Array,
    A_wqkv: jax.Array,
    A_wo: jax.Array,
    B_x: jax.Array,
    B_w_gate: jax.Array,
    B_w_up: jax.Array,
    B_w_down: jax.Array,
):
    del B_x
    anyspec = pl.BlockSpec(memory_space=pl.ANY)
    out = pl.pallas_call(
        _kernel,
        grid=(NTILE + 1,),
        in_specs=[anyspec] * 6,
        out_specs=anyspec,
        out_shape=jax.ShapeDtypeStruct((S, D), bf16),
        scratch_shapes=[
            pltpu.VMEM((S, D), bf16),
            pltpu.VMEM((D, 3 * D), bf16),
            pltpu.VMEM((D, D), bf16),
            pltpu.VMEM((FT * 128, D), bf16),
            pltpu.VMEM((FT * 128, D), bf16),
            pltpu.VMEM((2 * FR, D), bf16),
            pltpu.VMEM((F, D), bf16),
            pltpu.SemaphoreType.DMA((15,)),
            pltpu.VMEM((D, D), bf16),
            pltpu.VMEM((NG, S // 2, 128), u32),
            pltpu.VMEM((S // 128, H * 16, 128), u32),
            pltpu.VMEM((NG, T // 2, 128), u32),
            pltpu.VMEM((D, T), f32),
            pltpu.VMEM((KT, S, 128), bf16),
            pltpu.VMEM((T, D), bf16),
            pltpu.VMEM((T, D), f32),
            pltpu.VMEM((S, D), bf16),
            pltpu.SemaphoreType.DMA((NTILE - 1 + KT,)),
        ],
        compiler_params=pltpu.CompilerParams(dimension_semantics=("arbitrary",),
                                             vmem_limit_bytes=100 * 1024 * 1024),
    )(A_x.reshape(S, D), A_wqkv, A_wo, B_w_gate.T, B_w_up.T, B_w_down)
    return out.reshape(1, S, D)
```

```python
import math

import jax
import jax.numpy as jnp
from jax import lax
from jax.experimental import pallas as pl
from jax.experimental.pallas import tpu as pltpu

S, D, H, DH, W, F = 2048, 640, 32, 20, 256, 1728
f32 = jnp.float32
bf16 = jnp.bfloat16
u32 = jnp.uint32
NT = (((1,), (1,)), ((), ()))
NG = 8
NH = 4
SB = 32
NBLK = W // SB + 1
FT = F // 128
FR = F - FT * 128
KT = D // 128
NEG = -1e30
T = 256
NB = T // 128
NTILE = S // T

LAG, FILL, GATE, TAIL, PRE = 1, ((4, 4, 0), 7, (4, 4, 4)), (0, 4, 2), (8, (2, 2, 4)), 3
LAG0, FILL0, GATE0, TAIL0, PRE0 = 2, ((0, 0, 4), 10, (0, 4, 4)), (0, 0, 2), (4, (2, 2)), 1
KSPLIT, REGIONS, LN1_DUE, LN2_PACE, LAST_ROWS = 2, (20, 16, 52, 96), 8, (4, 2), 64


def _ln(x):
    m = jnp.mean(x, axis=-1, keepdims=True)
    xc = x - m
    v = jnp.mean(xc * xc, axis=-1, keepdims=True)
    return xc * lax.rsqrt(v + 1e-5)


def _sigmoid(x):
    return 0.5 * jnp.tanh(0.5 * x) + 0.5


def _pack(v):
    return pltpu.bitcast(v.astype(bf16), u32)


def _unpack(u):
    return pltpu.bitcast(u, bf16)


def _pull(gen, n):
    last = None
    for _ in range(n):
        v = next(gen, None)
        last = v if v is not None else last
    return last


def _mo(v, m):
    return v if isinstance(v, int) else pl.multiple_of(v, m)


def _chain(*gens):
    for g in gens:
        yield from g


def _take(g, n):
    for _ in range(n):
        yield next(g)


def _kernel(x_hbm, wqkv_hbm, wo_hbm, wg_hbm, wu_hbm, wd_hbm, o_hbm,
            x_ref, wqkv_ref, wo_ref, wg_ref, wu_ref, wt_ref, wd_ref, sem,
            wvt_ref, k_ref, vt_ref, q_ref, ot_ref, ln1_ref, ln2_ref, h_ref, o_ref, osem):
    step = pl.program_id(0)
    zero = step >> 10

    def copy(src, dst, n):
        return pltpu.make_async_copy(src, dst, sem.at[n])

    def rows(ref, r0, n):
        return ref.at[pl.ds(r0, n), :]

    def cols(ref, c0, n):
        return ref.at[:, pl.ds(c0, n)]

    def wcopy(c0, n, s):
        return copy(cols(wqkv_hbm, c0, n), cols(wqkv_ref, c0, n), s)

    def xcopy(r0, n, s):
        return copy(rows(x_hbm, r0, n), rows(x_ref, r0, n), s)

    lane_h = lax.broadcasted_iota(jnp.int32, (SB // 2, 128), 1)
    rr = lax.broadcasted_iota(jnp.int32, (SB, 128), 0)
    ll = lax.broadcasted_iota(jnp.int32, (SB, 128), 1)
    tri = rr <= (ll & (SB - 1))
    r8 = lax.broadcasted_iota(jnp.int32, (8, 128), 0)
    zero_u = jnp.zeros((SB // 2, 128), u32)
    never8 = r8 < zero
    never32 = rr < zero
    mk1 = (lane_h & SB) != 0
    mk2 = (lane_h & (2 * SB)) != 0

    pending = []

    def gated(v):
        hit = [p[1] for p in pending if p[0] == 0]
        pending[:] = [[p[0] - 1, p[1]] for p in pending if p[0] > 0]
        if not hit:
            return v
        u = pltpu.bitcast(v, u32)
        head = u[:8]
        for t in hit:
            head = jnp.where(never8, t, head)
        return _unpack(jnp.concatenate([head, u[8:]], axis=0))

    def after_tok(x, tok):
        return jnp.concatenate([jnp.where(never32, tok, x[:, :128]), x[:, 128:]], axis=1)

    def ln1_chunk(r, ch, tok=None, due=None):
        x = x_ref[r:r + ch, :].astype(f32)
        if tok is not None:
            x = after_tok(x, tok[:ch])
        y = _ln(x)
        if due is not None:
            t = y[0:8, 0:128]
            for s in range(8, ch, 8):
                t = t + y[s:s + 8, 0:128]
            pending.append([due, pltpu.bitcast(t, u32)])
        for k in range(KT):
            ln1_ref[k, r:r + ch, :] = y[:, k * 128:(k + 1) * 128].astype(bf16)

    def ln1_tile(tile, k, r0=0, n=T):
        return gated(ln1_ref[k, pl.ds(_mo(tile * T + r0, 128), n), :])

    def weave(gen, n, r0, nrows, every, free, due=None):
        todo = list(range(r0, r0 + nrows, SB))
        for _ in range(free):
            ln1_chunk(todo.pop(0), SB)
        for j in range(n):
            acc = next(gen)
            if todo and j % every == 0:
                ln1_chunk(todo.pop(0), SB, acc, due)
        assert not todo

    def proj_gen(tile, col0, store):
        lane_t = lax.broadcasted_iota(jnp.int32, (T, 128), 1)
        tiles = []
        done = 0
        for n in range(KT):
            acc = None
            for k in range(KT):
                p = jnp.dot(ln1_tile(tile, k),
                            wqkv_ref[k * 128:(k + 1) * 128, col0 + n * 128:col0 + (n + 1) * 128],
                            preferred_element_type=f32)
                acc = p if acc is None else p + acc
                if k == KT - 1:
                    tiles.append(acc)
                    while done < NG and (80 * done + 79) // 128 <= n:
                        lo = 80 * done
                        ta, tb = lo // 128, (lo + 79) // 128
                        a = tiles[ta]
                        if tb != ta:
                            a = jnp.where(lane_t >= lo % 128, a, tiles[tb])
                        store(done, a)
                        done += 1
                yield acc

    def k_gen(tile):
        def store(g, a):
            k_ref[g, tile * (T // 2):(tile + 1) * (T // 2), :] = _pack(a)
        return proj_gen(tile, D, store)

    def q_gen(tile):
        qscale = DH ** -0.5 * math.log2(math.e)

        def store(g, a):
            q_ref[g] = _pack(a * qscale)
        return proj_gen(tile, 0, store)

    def v_gen(tile):
        for b in range(NB):
            for hf in range(2):
                acc = None
                for k in range(KT):
                    p = lax.dot_general(wvt_ref[hf * 320:(hf + 1) * 320, k * 128:(k + 1) * 128],
                                        ln1_tile(tile, k, b * 128, 128), NT, preferred_element_type=f32)
                    acc = p if acc is None else p + acc
                    if k == KT - 1:
                        for h in range(hf * 16, hf * 16 + 16):
                            a = (5 * h) // 4 - hf * 20
                            o = 4 * (h % 4)
                            vh = jnp.where((rr >= o) & (rr < o + DH), acc[16 * a:16 * a + 32, :], 1.0)
                            vt_ref[tile * NB + b, h * 16:(h + 1) * 16, :] = _pack(vh)
                    yield acc

    def nskip(first, b, c):
        return max(0, (W - b * 128 - c * SB) // SB) if first else 0

    def stage_qk(first, hbase, b, g):
        res = {}
        for c in [(cc + (g if first else 0)) % NH for cc in range(NH)]:
            r0 = (b * 128 + c * SB) // 2
            q0 = _mo(hbase + r0, SB // 2)
            qs = q_ref[g, r0:r0 + SB // 2, :]
            wrows = []
            for j in range(NH):
                hh = 4 * g + (j ^ c)
                mk = ((lane_h - (20 * hh) % 128) & 127) < DH
                wrows.append(jnp.where(mk, qs, zero_u))
            wc = _unpack(jnp.concatenate(wrows, axis=0))
            ns = nskip(first, b, c)
            parts = [k_ref[g, pl.ds(q0, SB // 2), :]]
            if ns < 8:
                parts.append(k_ref[g, pl.ds(q0 - (W - ns * SB) // 2, (W - ns * SB) // 2), :])
            kw = jnp.concatenate(parts, axis=0) if len(parts) > 1 else parts[0]
            s = lax.dot_general(_unpack(kw), wc, NT, preferred_element_type=f32)
            if ns == 0:
                mrg = jnp.where(tri, s[:SB], s[SB:2 * SB])
                sm = jnp.concatenate([mrg, s[2 * SB:]], axis=0)
            else:
                mrg = jnp.where(tri, s[:SB], NEG)
                sm = jnp.concatenate([mrg, s[SB:]], axis=0) if ns < 8 else mrg
            m = jnp.max(jnp.max(sm.reshape(sm.shape[0] // 8, 8, 128), axis=0), axis=0, keepdims=True)
            res[c] = (sm, m)
        return res

    def sel(mk, hi, lo):
        if lo is None and hi is None:
            return None
        return jnp.where(mk, zero_u if hi is None else hi, zero_u if lo is None else lo)

    def stage_exp(first, b, sres, toks, gate):
        pm = [jnp.exp2(sres[c][0][:SB] - sres[c][1]) for c in range(NH)]
        rho0 = max(0, 8 - 4 * b) if first else 0
        pw = [{} for _ in range(NH)]
        blks = [[] for _ in range(NH)]
        for rho in range(rho0, 12):
            cur = []
            for c in range(NH):
                ns = nskip(first, b, c)
                sm, m = sres[c]
                j = rho - c
                if j < ns or j >= NBLK:
                    cur.append(None)
                elif j == NBLK - 1:
                    cur.append(_pack(jnp.where(tri, pm[c], 0.0) if ns == 0 else pm[c]))
                elif j == 0:
                    cur.append(_pack(jnp.where(tri, 0.0, pm[c])))
                else:
                    r0 = (j - ns + (1 if ns else 0)) * SB
                    if toks:
                        ntok = len(toks) * 32
                        pos = gate[0] + ((rho - rho0) * (ntok - gate[0] - gate[1])) // (12 - rho0)
                        tok = toks[pos // 32][(pos % 32) * 8:(pos % 32) * 8 + 8]
                        mg = jnp.where(never8, tok, jnp.broadcast_to(m, (8, 128)))
                        d = (sm[r0:r0 + SB].reshape(4, 8, 128) - mg[None]).reshape(SB, 128)
                    else:
                        d = sm[r0:r0 + SB] - m
                    cur.append(_pack(jnp.exp2(d)))
            cur = [sel(mk1, cur[e ^ 1], cur[e]) for e in range(NH)]
            cur = [sel(mk2, cur[e ^ 2], cur[e]) for e in range(NH)]
            for e in range(NH):
                blks[e].append(cur[e])
                if rho % 4 == 3:
                    pw[e][rho // 4] = _unpack(jnp.concatenate(blks[e], axis=0))
                    blks[e] = []
        return pw

    def stage_pv(blk, b, g, pw, after):
        vb = blk + b - 2
        res = [None] * NH
        for t in range(3):
            if t in pw[0]:
                for e in range(NH):
                    h = 4 * g + e
                    r = jnp.dot(_unpack(vt_ref[vb + t, h * 16:(h + 1) * 16, :]), pw[e][t],
                                preferred_element_type=f32)
                    res[e] = r if res[e] is None else r + res[e]
            after(t)
        outs = []
        for e in range(NH):
            r = res[e]
            if e < 2:
                inv = 1.0 / r[24:32]
                outs.append([r[8 * t:8 * t + 8] * inv for t in range(3)])
            else:
                inv = 1.0 / r[0:8]
                outs.append([r[8 * t:8 * t + 8] * inv for t in range(1, 4)])
        lo4 = r8 < 4
        rws = [outs[0][0], outs[0][1], jnp.where(lo4, outs[0][2], outs[1][0]), outs[1][1], outs[1][2],
               outs[2][0], outs[2][1], jnp.where(lo4, outs[2][2], outs[3][0]), outs[3][1], outs[3][2]]
        ot_ref[g * 80:(g + 1) * 80, b * 128:(b + 1) * 128] = jnp.concatenate(rws, axis=0)

    def attention(first, tile, gen, lag, fills, gate):
        units = [(b, g) for b in range(NB) for g in range(NG)]
        pws = []
        for u in range(len(units) + lag):
            if u < len(units):
                sres = stage_qk(first, tile * (T // 2), *units[u])
            toks = []
            fill = fills[0] if u < fills[1] else fills[2]

            def after(t):
                v = _pull(gen, fill[t])
                if v is not None and len(toks) < gate[2]:
                    toks.append(v)
            if u >= lag:
                stage_pv(tile * NB, *units[u - lag], pws[u - lag], after)
            else:
                for t in range(3):
                    after(t)
            if u < len(units):
                pws.append(stage_exp(first, units[u][0], sres, toks, gate))

    def out_proj(base, split):
        o_t = ot_ref[...].T
        lhs = []
        for t in range(KT):
            e_lane = ((lane_h + t * 128) // DH) % NH
            ob = _pack(o_t[:, t * 128:(t + 1) * 128])
            blks = [ob[r * 16:(r + 1) * 16, :] for r in range(T // SB)]
            for bit in (1, 2):
                mk = (e_lane & bit) != 0
                blks = [jnp.where(mk, blks[r ^ bit], blks[r]) for r in range(T // SB)]
            lhs.append(_unpack(jnp.concatenate(blks, axis=0)))
        outs = []
        cnt = 0
        for n in range(KT):
            acc = x_ref[pl.ds(base, T), n * 128:(n + 1) * 128].astype(f32)
            for k in range(KT):
                w = wo_ref[k * 128:(k + 1) * 128, n * 128:(n + 1) * 128]
                if cnt < len(split):
                    m = T // split[cnt]
                    acc = jnp.concatenate(
                        [jnp.dot(lhs[k][r:r + m], w, preferred_element_type=f32) + acc[r:r + m]
                         for r in range(0, T, m)], axis=0)
                else:
                    acc = jnp.dot(lhs[k], w, preferred_element_type=f32) + acc
                cnt += 1
            outs.append(acc)
        return jnp.concatenate(outs, axis=1)

    def finish(hres, gen):
        toks = []
        while True:
            v = _pull(gen, 4)
            if v is None:
                break
            toks.append(v)
        h_ref[...] = hres
        for c, r in enumerate(range(0, T, SB)):
            pos = LN2_PACE[0] + c * LN2_PACE[1]
            tok = toks[pos // 8][(pos % 8) * SB:(pos % 8 + 1) * SB]
            ln2_ref[r:r + SB, :] = _ln(after_tok(hres[r:r + SB], tok)).astype(bf16)

    def ffn_gen(tile, done=None):
        ln2 = [ln2_ref[:, k * 128:(k + 1) * 128] for k in range(KT)]
        acts = []

        def proj(w_ref, r0):
            acc = None
            for k in range(KT):
                p = lax.dot_general(ln2[k], w_ref[r0:r0 + 128, k * 128:(k + 1) * 128], NT,
                                    preferred_element_type=f32)
                acc = p if acc is None else p + acc
                if k == KT - 1:
                    res.append(acc)
                yield acc

        for j in range(FT):
            res = []
            yield from proj(wg_ref, j * 128)
            yield from proj(wu_ref, j * 128)
            acts.append(_sigmoid(res[0]) * res[1])
        res = []
        yield from proj(wt_ref, 0)
        acts.append((_sigmoid(res[0]) * pltpu.roll(res[0], FR, 1))[:, :FR])
        cache = {}

        def act(j, ra, nr):
            if (j, ra, nr) not in cache:
                cache[j, ra, nr] = acts[j][ra:ra + nr].astype(bf16)
            return cache[j, ra, nr]

        pieces = [(n, 0, T) for n in range(KT)]
        if done is not None:
            pieces = pieces[:-1] + [(KT - 1, 0, T - LAST_ROWS), (KT - 1, T - LAST_ROWS, LAST_ROWS)]
        for idx, (n, ra, nr) in enumerate(pieces):
            acc = h_ref[ra:ra + nr, n * 128:(n + 1) * 128]
            for j in range(FT + 1):
                r1 = min(F, (j + 1) * 128)
                acc = jnp.dot(act(j, ra, nr), wd_ref[j * 128:r1, n * 128:(n + 1) * 128],
                              preferred_element_type=f32) + acc
                if j == FT:
                    o_ref[pl.ds(_mo(tile * T + ra, 16), nr), n * 128:(n + 1) * 128] = acc.astype(o_ref.dtype)
                    if done is not None:
                        done(idx, n, ra, nr)
                yield acc

    def ocopy(tile):
        r0 = _mo(tile * T, T)
        return pltpu.make_async_copy(rows(o_ref, r0, T), rows(o_hbm, r0, T), osem.at[tile])

    def ocopy_last(idx, n, ra, nr):
        sl = (pl.ds(S - T + ra, nr), pl.ds(n * 128, 128))
        return pltpu.make_async_copy(o_ref.at[sl], o_hbm.at[sl], osem.at[NTILE - 1 + idx])

    def prologue():
        ka = 128 * KSPLIT
        cp_x0, cp_x1 = xcopy(0, T, 0), xcopy(T, T, 1)
        cp_ka, cp_kb = wcopy(D, ka, 2), wcopy(D + ka, D - ka, 3)
        cp_v, cp_q = wcopy(2 * D, D, 4), wcopy(0, D, 5)
        cp_o = copy(wo_hbm, wo_ref, 6)
        cp_ffn = [copy(rows(wg_hbm, 0, FT * 128), wg_ref, 7), copy(rows(wu_hbm, 0, FT * 128), wu_ref, 8),
                  copy(rows(wg_hbm, FT * 128, FR), rows(wt_ref, 0, FR), 9),
                  copy(rows(wu_hbm, FT * 128, FR), rows(wt_ref, FR, FR), 10),
                  copy(wd_hbm, wd_ref, 11)]
        cp_xs = [xcopy(2 * T * (j + 1), 2 * T, 12 + j) for j in range(3)]
        for cp in [cp_x0, cp_x1, cp_ka, cp_kb, cp_xs[0], cp_v, cp_xs[1], cp_q, cp_xs[2], cp_o] + cp_ffn:
            cp.start()
        cp_x0.wait()
        ln1_chunk(0, T)
        cp_x1.wait()
        ln1_chunk(T, T)
        g0, g1, g6 = k_gen(0), k_gen(1), k_gen(6)
        gen = _chain(_take(g0, KSPLIT * KT), _take(g1, KSPLIT * KT), g0, g1, k_gen(2), k_gen(3),
                     v_gen(0), v_gen(1), k_gen(4), k_gen(5), v_gen(2), v_gen(3), q_gen(0),
                     _take(g6, 1), v_gen(4), v_gen(5), v_gen(6), v_gen(7), g6, k_gen(7))
        n1, n2, n3, n4 = REGIONS
        cp_ka.wait()
        _pull(gen, n1)
        cp_kb.wait()
        _pull(gen, n2)
        cp_xs[0].wait()
        left = 50 - n1 - n2
        weave(gen, left, 2 * T, T, 2, 2)
        weave(gen, 25, 3 * T, T, 3, 0)
        _pull(gen, n3 - left - 25)
        cp_v.wait()
        cp_xs[1].wait()
        wvt_ref[...] = wqkv_ref[:, 2 * D:].T
        left = 100 - n1 - n2 - n3
        _pull(gen, left)
        weave(gen, 40, 4 * T, T, 4, 0, LN1_DUE)
        weave(gen, 25, 5 * T, T, 3, 0, LN1_DUE)
        _pull(gen, n4 - left - 65)
        cp_q.wait()
        cp_xs[2].wait()
        cp_o.wait()
        left = 230 - n1 - n2 - n3 - n4
        weave(gen, left + 25, 6 * T, 2 * T, 4, 0, LN1_DUE)
        _pull(gen, PRE0)
        attention(True, 0, gen, LAG0, FILL0, GATE0)
        _pull(gen, TAIL0[0])
        hres = out_proj(0, TAIL0[1])
        finish(hres, gen)
        for cp in cp_ffn:
            cp.wait()

    def body(i, carry):
        _pull(q_gen(i), 100)
        gen = ffn_gen(i - 1)
        _pull(gen, PRE)
        attention(False, i, gen, LAG, FILL, GATE)
        _pull(gen, TAIL[0])
        hres = out_proj(pl.multiple_of(i * T, T), TAIL[1])
        finish(hres, gen)
        ocopy(i - 1).start()
        return carry

    def epilogue():
        cps = []

        def done(*a):
            cps.append(ocopy_last(*a))
            cps[-1].start()
        _pull(ffn_gen(NTILE - 1, done), 1000)
        for t in range(NTILE - 1):
            ocopy(t).wait()
        for cp in cps:
            cp.wait()

    @pl.when(step == 0)
    def _():
        prologue()
        lax.fori_loop(1, NTILE, body, 0)
        epilogue()


@jax.jit
def pallas_sequential_preLN__sliding_block__glu_gated_glu__prompt_kernel(
    A_x: jax.Array,
    A_wqkv: jax.Array,
    A_wo: jax.Array,
    B_x: jax.Array,
    B_w_gate: jax.Array,
    B_w_up: jax.Array,
    B_w_down: jax.Array,
):
    del B_x
    anyspec = pl.BlockSpec(memory_space=pl.ANY)
    out = pl.pallas_call(
        _kernel,
        grid=(2,),
        in_specs=[anyspec] * 6,
        out_specs=anyspec,
        out_shape=jax.ShapeDtypeStruct((S, D), bf16),
        scratch_shapes=[
            pltpu.VMEM((S, D), bf16),
            pltpu.VMEM((D, 3 * D), bf16),
            pltpu.VMEM((D, D), bf16),
            pltpu.VMEM((FT * 128, D), bf16),
            pltpu.VMEM((FT * 128, D), bf16),
            pltpu.VMEM((2 * FR, D), bf16),
            pltpu.VMEM((F, D), bf16),
            pltpu.SemaphoreType.DMA((15,)),
            pltpu.VMEM((D, D), bf16),
            pltpu.VMEM((NG, S // 2, 128), u32),
            pltpu.VMEM((S // 128, H * 16, 128), u32),
            pltpu.VMEM((NG, T // 2, 128), u32),
            pltpu.VMEM((D, T), f32),
            pltpu.VMEM((KT, S, 128), bf16),
            pltpu.VMEM((T, D), bf16),
            pltpu.VMEM((T, D), f32),
            pltpu.VMEM((S, D), bf16),
            pltpu.SemaphoreType.DMA((NTILE + KT,)),
        ],
        compiler_params=pltpu.CompilerParams(dimension_semantics=("arbitrary",),
                                             vmem_limit_bytes=100 * 1024 * 1024),
    )(A_x.reshape(S, D), A_wqkv, A_wo, B_w_gate.T, B_w_up.T, B_w_down)
    return out.reshape(1, S, D)
```

```python
import math

import jax
import jax.numpy as jnp
from jax import lax
from jax.experimental import pallas as pl
from jax.experimental.pallas import tpu as pltpu

S, D, H, DH, W, F = 2048, 640, 32, 20, 256, 1728
f32 = jnp.float32
bf16 = jnp.bfloat16
u32 = jnp.uint32
NN = (((1,), (0,)), ((), ()))
NT = (((1,), (1,)), ((), ()))
NG = 8
NH = 4
SB = 32
NBLK = W // SB + 1
FT = F // 128
FR = F - FT * 128
KT = D // 128
NEG = -1e30
T = 256
NB = T // 128
NTILE = S // T

LAG, FILL, GATE, TAIL, PRE = 1, ((4, 4, 0), 7, (4, 4, 4)), (0, 4, 2), (4, (2, 2, 4)), 3
LAG0, FILL0, GATE0, TAIL0, PRE0 = 2, ((0, 0, 4), 10, (0, 4, 4)), (0, 0, 2), (4, (2, 2)), 1
KSPLIT, REGIONS, LN1_DUE, LN2_PACE, LAST_ROWS = 2, (20, 16, 52, 96), 8, (4, 2), 64


def _ln(x):
    m = jnp.mean(x, axis=-1, keepdims=True)
    xc = x - m
    v = jnp.mean(xc * xc, axis=-1, keepdims=True)
    return xc * lax.rsqrt(v + 1e-5)


def _sigmoid(x):
    return 0.5 * jnp.tanh(0.5 * x) + 0.5


def _pack(v):
    return pltpu.bitcast(v.astype(bf16), u32)


def _unpack(u):
    return pltpu.bitcast(u, bf16)


def _pull(gen, n):
    last = None
    for _ in range(n):
        v = next(gen, None)
        last = v if v is not None else last
    return last


def _mo(v, m):
    return v if isinstance(v, int) else pl.multiple_of(v, m)


def _chain(*gens):
    for g in gens:
        yield from g


def _take(g, n):
    for _ in range(n):
        yield next(g)


def _kernel(x_hbm, wqkv_hbm, wo_hbm, wg_hbm, wu_hbm, wd_hbm, o_hbm,
            x_ref, wqkv_ref, wo_ref, wg_ref, wu_ref, wt_ref, wd_ref, sem,
            wvt_ref, k_ref, vt_ref, q_ref, ot_ref, ln1_ref, ln2_ref, h_ref, o_ref, osem):
    step = pl.program_id(0)
    zero = step >> 10

    def copy(src, dst, n):
        return pltpu.make_async_copy(src, dst, sem.at[n])

    def rows(ref, r0, n):
        return ref.at[pl.ds(r0, n), :]

    def cols(ref, c0, n):
        return ref.at[:, pl.ds(c0, n)]

    def wcopy(c0, n, s):
        return copy(cols(wqkv_hbm, c0, n), cols(wqkv_ref, c0, n), s)

    def xcopy(r0, n, s):
        return copy(rows(x_hbm, r0, n), rows(x_ref, r0, n), s)

    lane_h = lax.broadcasted_iota(jnp.int32, (SB // 2, 128), 1)
    rr = lax.broadcasted_iota(jnp.int32, (SB, 128), 0)
    ll = lax.broadcasted_iota(jnp.int32, (SB, 128), 1)
    tri = rr <= (ll & (SB - 1))
    r8 = lax.broadcasted_iota(jnp.int32, (8, 128), 0)
    zero_u = jnp.zeros((SB // 2, 128), u32)
    lo4 = r8 < 4
    never8 = r8 < zero
    never32 = rr < zero
    mk1 = (lane_h & SB) != 0
    mk2 = (lane_h & (2 * SB)) != 0

    pending = []

    def gated(v):
        hit = [p[1] for p in pending if p[0] == 0]
        pending[:] = [[p[0] - 1, p[1]] for p in pending if p[0] > 0]
        if not hit:
            return v
        u = pltpu.bitcast(v, u32)
        head = u[:8]
        for t in hit:
            head = jnp.where(never8, t, head)
        return _unpack(jnp.concatenate([head, u[8:]], axis=0))

    def after_tok(x, tok):
        return jnp.concatenate([jnp.where(never32, tok, x[:, :128]), x[:, 128:]], axis=1)

    def ln1_chunk(r, ch, tok=None, due=None):
        x = x_ref[r:r + ch, :].astype(f32)
        if tok is not None:
            x = after_tok(x, tok[:ch])
        y = _ln(x)
        if due is not None:
            t = y[0:8, 0:128]
            for s in range(8, ch, 8):
                t = t + y[s:s + 8, 0:128]
            pending.append([due, pltpu.bitcast(t, u32)])
        for k in range(KT):
            ln1_ref[k, r:r + ch, :] = y[:, k * 128:(k + 1) * 128].astype(bf16)

    def ln1_tile(tile, k, r0=0, n=T):
        return gated(ln1_ref[k, pl.ds(_mo(tile * T + r0, 128), n), :])

    def weave(gen, n, r0, nrows, every, free, due=None):
        todo = list(range(r0, r0 + nrows, SB))
        for _ in range(free):
            ln1_chunk(todo.pop(0), SB)
        for j in range(n):
            acc = next(gen)
            if todo and j % every == 0:
                ln1_chunk(todo.pop(0), SB, acc, due)
        assert not todo

    def proj_gen(tile, col0, store):
        lane_t = lax.broadcasted_iota(jnp.int32, (T, 128), 1)
        tiles = []
        done = 0
        for n in range(KT):
            acc = None
            for k in range(KT):
                p = jnp.dot(ln1_tile(tile, k),
                            wqkv_ref[k * 128:(k + 1) * 128, col0 + n * 128:col0 + (n + 1) * 128],
                            preferred_element_type=f32)
                acc = p if acc is None else p + acc
                if k == KT - 1:
                    tiles.append(acc)
                    while done < NG and (80 * done + 79) // 128 <= n:
                        lo = 80 * done
                        ta, tb = lo // 128, (lo + 79) // 128
                        a = tiles[ta]
                        if tb != ta:
                            a = jnp.where(lane_t >= lo % 128, a, tiles[tb])
                        store(done, a)
                        done += 1
                yield acc

    def k_gen(tile):
        def store(g, a):
            k_ref[g, tile * (T // 2):(tile + 1) * (T // 2), :] = _pack(a)
        return proj_gen(tile, D, store)

    def q_gen(tile):
        qscale = DH ** -0.5 * math.log2(math.e)

        def store(g, a):
            q_ref[g] = _pack(a * qscale)
        return proj_gen(tile, 0, store)

    def v_gen(tile):
        for b in range(NB):
            for hf in range(2):
                acc = None
                for k in range(KT):
                    p = lax.dot_general(wvt_ref[hf * 320:(hf + 1) * 320, k * 128:(k + 1) * 128],
                                        ln1_tile(tile, k, b * 128, 128), NT, preferred_element_type=f32)
                    acc = p if acc is None else p + acc
                    if k == KT - 1:
                        for h in range(hf * 16, hf * 16 + 16):
                            a = 8 * ((5 * h) // 2 - hf * 40)
                            if h % 2 == 0:
                                vh = [acc[a:a + 16], jnp.where(lo4, acc[a + 16:a + 24], 1.0)]
                            else:
                                vh = [jnp.where(lo4, 1.0, acc[a:a + 8]), acc[a + 8:a + 24]]
                            vt_ref[tile * NB + b, h * 24:(h + 1) * 24, :] = jnp.concatenate(vh, axis=0)
                    yield acc

    def nskip(first, b, c):
        return max(0, (W - b * 128 - c * SB) // SB) if first else 0

    def stage_qk(first, hbase, b, g):
        res = {}
        for c in [(cc + (g if first else 0)) % NH for cc in range(NH)]:
            r0 = (b * 128 + c * SB) // 2
            q0 = _mo(hbase + r0, SB // 2)
            qs = q_ref[g, r0:r0 + SB // 2, :]
            wrows = []
            for j in range(NH):
                hh = 4 * g + (j ^ c)
                mk = ((lane_h - (20 * hh) % 128) & 127) < DH
                wrows.append(jnp.where(mk, qs, zero_u))
            wc = _unpack(jnp.concatenate(wrows, axis=0))
            ns = nskip(first, b, c)
            parts = [k_ref[g, pl.ds(q0, SB // 2), :]]
            if ns < 8:
                parts.append(k_ref[g, pl.ds(q0 - (W - ns * SB) // 2, (W - ns * SB) // 2), :])
            kw = jnp.concatenate(parts, axis=0) if len(parts) > 1 else parts[0]
            s = lax.dot_general(_unpack(kw), wc, NT, preferred_element_type=f32)
            if ns == 0:
                mrg = jnp.where(tri, s[:SB], s[SB:2 * SB])
                sm = jnp.concatenate([mrg, s[2 * SB:]], axis=0)
            else:
                mrg = jnp.where(tri, s[:SB], NEG)
                sm = jnp.concatenate([mrg, s[SB:]], axis=0) if ns < 8 else mrg
            m = jnp.max(jnp.max(sm.reshape(sm.shape[0] // 8, 8, 128), axis=0), axis=0, keepdims=True)
            res[c] = (sm, m)
        return res

    def sel(mk, hi, lo):
        if lo is None and hi is None:
            return None
        return jnp.where(mk, zero_u if hi is None else hi, zero_u if lo is None else lo)

    def stage_exp(first, b, sres, toks, gate):
        pm = [jnp.exp2(sres[c][0][:SB] - sres[c][1]) for c in range(NH)]
        rho0 = max(0, 8 - 4 * b) if first else 0
        pw = [{} for _ in range(NH)]
        blks = [[] for _ in range(NH)]
        for rho in range(rho0, 12):
            cur = []
            for c in range(NH):
                ns = nskip(first, b, c)
                sm, m = sres[c]
                j = rho - c
                if j < ns or j >= NBLK:
                    cur.append(None)
                elif j == NBLK - 1:
                    cur.append(_pack(jnp.where(tri, pm[c], 0.0) if ns == 0 else pm[c]))
                elif j == 0:
                    cur.append(_pack(jnp.where(tri, 0.0, pm[c])))
                else:
                    r0 = (j - ns + (1 if ns else 0)) * SB
                    if toks:
                        ntok = len(toks) * 32
                        pos = gate[0] + ((rho - rho0) * (ntok - gate[0] - gate[1])) // (12 - rho0)
                        tok = toks[pos // 32][(pos % 32) * 8:(pos % 32) * 8 + 8]
                        mg = jnp.where(never8, tok, jnp.broadcast_to(m, (8, 128)))
                        d = (sm[r0:r0 + SB].reshape(4, 8, 128) - mg[None]).reshape(SB, 128)
                    else:
                        d = sm[r0:r0 + SB] - m
                    cur.append(_pack(jnp.exp2(d)))
            cur = [sel(mk1, cur[e ^ 1], cur[e]) for e in range(NH)]
            cur = [sel(mk2, cur[e ^ 2], cur[e]) for e in range(NH)]
            for e in range(NH):
                blks[e].append(cur[e])
                if rho % 4 == 3:
                    pw[e][rho // 4] = _unpack(jnp.concatenate(blks[e], axis=0))
                    blks[e] = []
        return pw

    def stage_pv(blk, b, g, pw, after):
        vb = blk + b - 2
        res = [None] * NH
        for t in range(3):
            if t in pw[0]:
                for e in range(NH):
                    h = 4 * g + e
                    r = lax.dot_general(vt_ref[vb + t, h * 24:(h + 1) * 24, :], pw[e][t], NN,
                                        preferred_element_type=f32)
                    res[e] = r if res[e] is None else r + res[e]
            after(t)
        rws = []
        for e in (0, 2):
            ev, od = res[e], res[e + 1]
            inv = 1.0 / jnp.where(lo4, od[0:8], ev[16:24])
            rol = pltpu.roll(inv, 4, 0)
            inv_e = jnp.where(lo4, rol, inv)
            inv_o = jnp.where(lo4, inv, rol)
            rws += [ev[0:8] * inv_e, ev[8:16] * inv_e, jnp.where(lo4, ev[16:24], od[0:8]) * rol,
                    od[8:16] * inv_o, od[16:24] * inv_o]
        ot_ref[g * 80:(g + 1) * 80, b * 128:(b + 1) * 128] = jnp.concatenate(rws, axis=0)

    def attention(first, tile, gen, lag, fills, gate):
        units = [(b, g) for b in range(NB) for g in range(NG)]
        pws = []
        for u in range(len(units) + lag):
            if u < len(units):
                sres = stage_qk(first, tile * (T // 2), *units[u])
            toks = []
            fill = fills[0] if u < fills[1] else fills[2]

            def after(t):
                v = _pull(gen, fill[t])
                if v is not None and len(toks) < gate[2]:
                    toks.append(v)
            if u >= lag:
                stage_pv(tile * NB, *units[u - lag], pws[u - lag], after)
            else:
                for t in range(3):
                    after(t)
            if u < len(units):
                pws.append(stage_exp(first, units[u][0], sres, toks, gate))

    def out_proj(base, split):
        o_t = ot_ref[...].T
        lhs = []
        for t in range(KT):
            e_lane = ((lane_h + t * 128) // DH) % NH
            ob = _pack(o_t[:, t * 128:(t + 1) * 128])
            blks = [ob[r * 16:(r + 1) * 16, :] for r in range(T // SB)]
            for bit in (1, 2):
                mk = (e_lane & bit) != 0
                blks = [jnp.where(mk, blks[r ^ bit], blks[r]) for r in range(T // SB)]
            lhs.append(_unpack(jnp.concatenate(blks, axis=0)))
        outs = []
        cnt = 0
        for n in range(KT):
            acc = x_ref[pl.ds(base, T), n * 128:(n + 1) * 128].astype(f32)
            for k in range(KT):
                w = wo_ref[k * 128:(k + 1) * 128, n * 128:(n + 1) * 128]
                if cnt < len(split):
                    m = T // split[cnt]
                    acc = jnp.concatenate(
                        [jnp.dot(lhs[k][r:r + m], w, preferred_element_type=f32) + acc[r:r + m]
                         for r in range(0, T, m)], axis=0)
                else:
                    acc = jnp.dot(lhs[k], w, preferred_element_type=f32) + acc
                cnt += 1
            outs.append(acc)
        return jnp.concatenate(outs, axis=1)

    def finish(hres, gen):
        toks = []
        while True:
            v = _pull(gen, 4)
            if v is None:
                break
            toks.append(v)
        h_ref[...] = hres
        for c, r in enumerate(range(0, T, SB)):
            pos = LN2_PACE[0] + c * LN2_PACE[1]
            tok = toks[pos // 8][(pos % 8) * SB:(pos % 8 + 1) * SB]
            ln2_ref[r:r + SB, :] = _ln(after_tok(hres[r:r + SB], tok)).astype(bf16)

    def ffn_gen(tile, done=None):
        ln2 = [ln2_ref[:, k * 128:(k + 1) * 128] for k in range(KT)]
        acts = []

        def proj(w_ref, r0):
            acc = None
            for k in range(KT):
                p = lax.dot_general(ln2[k], w_ref[r0:r0 + 128, k * 128:(k + 1) * 128], NT,
                                    preferred_element_type=f32)
                acc = p if acc is None else p + acc
                if k == KT - 1:
                    res.append(acc)
                yield acc

        for j in range(FT):
            res = []
            yield from proj(wg_ref, j * 128)
            yield from proj(wu_ref, j * 128)
            acts.append(_sigmoid(res[0]) * res[1])
        res = []
        yield from proj(wt_ref, 0)
        acts.append((_sigmoid(res[0]) * pltpu.roll(res[0], FR, 1))[:, :FR])
        cache = {}

        def act(j, ra, nr):
            if (j, ra, nr) not in cache:
                cache[j, ra, nr] = acts[j][ra:ra + nr].astype(bf16)
            return cache[j, ra, nr]

        pieces = [(n, 0, T) for n in range(KT)]
        if done is not None:
            pieces = pieces[:-1] + [(KT - 1, 0, T - LAST_ROWS), (KT - 1, T - LAST_ROWS, LAST_ROWS)]
        for idx, (n, ra, nr) in enumerate(pieces):
            acc = h_ref[ra:ra + nr, n * 128:(n + 1) * 128]
            for j in range(FT + 1):
                r1 = min(F, (j + 1) * 128)
                acc = jnp.dot(act(j, ra, nr), wd_ref[j * 128:r1, n * 128:(n + 1) * 128],
                              preferred_element_type=f32) + acc
                if j == FT:
                    o_ref[pl.ds(_mo(tile * T + ra, 16), nr), n * 128:(n + 1) * 128] = acc.astype(o_ref.dtype)
                    if done is not None:
                        done(idx, n, ra, nr)
                yield acc

    def ocopy(tile):
        r0 = _mo(tile * T, T)
        return pltpu.make_async_copy(rows(o_ref, r0, T), rows(o_hbm, r0, T), osem.at[tile])

    def ocopy_last(idx, n, ra, nr):
        sl = (pl.ds(S - T + ra, nr), pl.ds(n * 128, 128))
        return pltpu.make_async_copy(o_ref.at[sl], o_hbm.at[sl], osem.at[NTILE - 1 + idx])

    def prologue():
        ka = 128 * KSPLIT
        cp_x0, cp_x1 = xcopy(0, T, 0), xcopy(T, T, 1)
        cp_ka, cp_kb = wcopy(D, ka, 2), wcopy(D + ka, D - ka, 3)
        cp_v, cp_q = wcopy(2 * D, D, 4), wcopy(0, D, 5)
        cp_o = copy(wo_hbm, wo_ref, 6)
        cp_ffn = [copy(rows(wg_hbm, 0, FT * 128), wg_ref, 7), copy(rows(wu_hbm, 0, FT * 128), wu_ref, 8),
                  copy(rows(wg_hbm, FT * 128, FR), rows(wt_ref, 0, FR), 9),
                  copy(rows(wu_hbm, FT * 128, FR), rows(wt_ref, FR, FR), 10),
                  copy(wd_hbm, wd_ref, 11)]
        cp_xs = [xcopy(2 * T * (j + 1), 2 * T, 12 + j) for j in range(3)]
        for cp in [cp_x0, cp_x1, cp_ka, cp_kb, cp_xs[0], cp_v, cp_xs[1], cp_q, cp_xs[2], cp_o] + cp_ffn:
            cp.start()
        cp_x0.wait()
        ln1_chunk(0, T)
        cp_x1.wait()
        ln1_chunk(T, T)
        g0, g1, g6 = k_gen(0), k_gen(1), k_gen(6)
        gen = _chain(_take(g0, KSPLIT * KT), _take(g1, KSPLIT * KT), g0, g1, k_gen(2), k_gen(3),
                     v_gen(0), v_gen(1), k_gen(4), k_gen(5), v_gen(2), v_gen(3), q_gen(0),
                     _take(g6, 1), v_gen(4), v_gen(5), v_gen(6), v_gen(7), g6, k_gen(7))
        n1, n2, n3, n4 = REGIONS
        cp_ka.wait()
        _pull(gen, n1)
        cp_kb.wait()
        _pull(gen, n2)
        cp_xs[0].wait()
        left = 50 - n1 - n2
        weave(gen, left, 2 * T, T, 2, 2)
        weave(gen, 25, 3 * T, T, 3, 0)
        _pull(gen, n3 - left - 25)
        cp_v.wait()
        cp_xs[1].wait()
        wvt_ref[...] = wqkv_ref[:, 2 * D:].T
        left = 100 - n1 - n2 - n3
        _pull(gen, left)
        weave(gen, 40, 4 * T, T, 4, 0, LN1_DUE)
        weave(gen, 25, 5 * T, T, 3, 0, LN1_DUE)
        _pull(gen, n4 - left - 65)
        cp_q.wait()
        cp_xs[2].wait()
        cp_o.wait()
        left = 230 - n1 - n2 - n3 - n4
        weave(gen, left + 25, 6 * T, 2 * T, 4, 0, LN1_DUE)
        _pull(gen, PRE0)
        attention(True, 0, gen, LAG0, FILL0, GATE0)
        _pull(gen, TAIL0[0])
        hres = out_proj(0, TAIL0[1])
        finish(hres, gen)
        for cp in cp_ffn:
            cp.wait()

    def body(i, carry):
        _pull(q_gen(i), 100)
        gen = ffn_gen(i - 1)
        _pull(gen, PRE)
        attention(False, i, gen, LAG, FILL, GATE)
        _pull(gen, TAIL[0])
        hres = out_proj(pl.multiple_of(i * T, T), TAIL[1])
        finish(hres, gen)
        ocopy(i - 1).start()
        return carry

    def epilogue():
        cps = []

        def done(*a):
            cps.append(ocopy_last(*a))
            cps[-1].start()
        _pull(ffn_gen(NTILE - 1, done), 1000)
        for t in range(NTILE - 1):
            ocopy(t).wait()
        for cp in cps:
            cp.wait()

    @pl.when(step == 0)
    def _():
        prologue()
        lax.fori_loop(1, NTILE, body, 0)
        epilogue()


@jax.jit
def pallas_sequential_preLN__sliding_block__glu_gated_glu__prompt_kernel(
    A_x: jax.Array,
    A_wqkv: jax.Array,
    A_wo: jax.Array,
    B_x: jax.Array,
    B_w_gate: jax.Array,
    B_w_up: jax.Array,
    B_w_down: jax.Array,
):
    del B_x
    anyspec = pl.BlockSpec(memory_space=pl.ANY)
    out = pl.pallas_call(
        _kernel,
        grid=(2,),
        in_specs=[anyspec] * 6,
        out_specs=anyspec,
        out_shape=jax.ShapeDtypeStruct((S, D), bf16),
        scratch_shapes=[
            pltpu.VMEM((S, D), bf16),
            pltpu.VMEM((D, 3 * D), bf16),
            pltpu.VMEM((D, D), bf16),
            pltpu.VMEM((FT * 128, D), bf16),
            pltpu.VMEM((FT * 128, D), bf16),
            pltpu.VMEM((2 * FR, D), bf16),
            pltpu.VMEM((F, D), bf16),
            pltpu.SemaphoreType.DMA((15,)),
            pltpu.VMEM((D, D), bf16),
            pltpu.VMEM((NG, S // 2, 128), u32),
            pltpu.VMEM((S // 128, H * 24, 128), f32),
            pltpu.VMEM((NG, T // 2, 128), u32),
            pltpu.VMEM((D, T), f32),
            pltpu.VMEM((KT, S, 128), bf16),
            pltpu.VMEM((T, D), bf16),
            pltpu.VMEM((T, D), f32),
            pltpu.VMEM((S, D), bf16),
            pltpu.SemaphoreType.DMA((NTILE + KT,)),
        ],
        compiler_params=pltpu.CompilerParams(dimension_semantics=("arbitrary",),
                                             vmem_limit_bytes=100 * 1024 * 1024),
    )(A_x.reshape(S, D), A_wqkv, A_wo, B_w_gate.T, B_w_up.T, B_w_down)
    return out.reshape(1, S, D)
```

```python
import math

import jax
import jax.numpy as jnp
from jax import lax
from jax.experimental import pallas as pl
from jax.experimental.pallas import tpu as pltpu

S, D, H, DH, W, F = 2048, 640, 32, 20, 256, 1728
f32 = jnp.float32
bf16 = jnp.bfloat16
u32 = jnp.uint32
NN = (((1,), (0,)), ((), ()))
NT = (((1,), (1,)), ((), ()))
NG = 8
NH = 4
SB = 32
NBLK = W // SB + 1
FT = F // 128
FR = F - FT * 128
KT = D // 128
NEG = -1e30
T = 256
NB = T // 128
NTILE = S // T

LAG, FILL, GATE, TAIL, PRE, PACE = 1, ((4, 4, 0), 7, (4, 4, 4)), (0, 4, 2), (4, (2, 2, 4)), 3, (4, 2)
LAG0, FILL0, GATE0, TAIL0, PRE0, PACE0 = 2, ((0, 0, 4), 10, (0, 4, 4)), (0, 0, 2), (4, (2, 2)), 1, (0, 3)
KSPLIT, REGIONS, LN1_DUE, LAST_ROWS = 2, (20, 16, 52, 96), 8, 64


def _ln(x):
    m = jnp.mean(x, axis=-1, keepdims=True)
    xc = x - m
    v = jnp.mean(xc * xc, axis=-1, keepdims=True)
    return xc * lax.rsqrt(v + 1e-5)


def _sigmoid(x):
    return 0.5 * jnp.tanh(0.5 * x) + 0.5


def _pack(v):
    return pltpu.bitcast(v.astype(bf16), u32)


def _unpack(u):
    return pltpu.bitcast(u, bf16)


def _pull(gen, n):
    last = None
    for _ in range(n):
        v = next(gen, None)
        last = v if v is not None else last
    return last


def _mo(v, m):
    return v if isinstance(v, int) else pl.multiple_of(v, m)


def _chain(*gens):
    for g in gens:
        yield from g


def _take(g, n):
    for _ in range(n):
        yield next(g)


def _kernel(x_hbm, wqkv_hbm, wo_hbm, wg_hbm, wu_hbm, wd_hbm, o_hbm,
            x_ref, wqkv_ref, wo_ref, wg_ref, wu_ref, wt_ref, wd_ref, sem,
            wvt_ref, k_ref, vt_ref, q_ref, ot_ref, ln1_ref, ln2_ref, h_ref, o_ref, osem):
    step = pl.program_id(0)
    zero = step >> 10

    def copy(src, dst, n):
        return pltpu.make_async_copy(src, dst, sem.at[n])

    def rows(ref, r0, n):
        return ref.at[pl.ds(r0, n), :]

    def cols(ref, c0, n):
        return ref.at[:, pl.ds(c0, n)]

    def wcopy(c0, n, s):
        return copy(cols(wqkv_hbm, c0, n), cols(wqkv_ref, c0, n), s)

    def xcopy(r0, n, s):
        return copy(rows(x_hbm, r0, n), rows(x_ref, r0, n), s)

    lane_h = lax.broadcasted_iota(jnp.int32, (SB // 2, 128), 1)
    rr = lax.broadcasted_iota(jnp.int32, (SB, 128), 0)
    ll = lax.broadcasted_iota(jnp.int32, (SB, 128), 1)
    tri = rr <= (ll & (SB - 1))
    r8 = lax.broadcasted_iota(jnp.int32, (8, 128), 0)
    zero_u = jnp.zeros((SB // 2, 128), u32)
    lo4 = r8 < 4
    never8 = r8 < zero
    never32 = rr < zero
    mk1 = (lane_h & SB) != 0
    mk2 = (lane_h & (2 * SB)) != 0

    pending = []

    def gated(v):
        hit = [p[1] for p in pending if p[0] == 0]
        pending[:] = [[p[0] - 1, p[1]] for p in pending if p[0] > 0]
        if not hit:
            return v
        u = pltpu.bitcast(v, u32)
        head = u[:8]
        for t in hit:
            head = jnp.where(never8, t, head)
        return _unpack(jnp.concatenate([head, u[8:]], axis=0))

    def after_tok(x, tok):
        return jnp.concatenate([jnp.where(never32, tok, x[:, :128]), x[:, 128:]], axis=1)

    def ln1_chunk(r, ch, tok=None, due=None):
        x = x_ref[r:r + ch, :].astype(f32)
        if tok is not None:
            x = after_tok(x, tok[:ch])
        y = _ln(x)
        if due is not None:
            t = y[0:8, 0:128]
            for s in range(8, ch, 8):
                t = t + y[s:s + 8, 0:128]
            pending.append([due, pltpu.bitcast(t, u32)])
        for k in range(KT):
            ln1_ref[k, r:r + ch, :] = y[:, k * 128:(k + 1) * 128].astype(bf16)

    def ln1_tile(tile, k, r0=0, n=T):
        return gated(ln1_ref[k, pl.ds(_mo(tile * T + r0, 128), n), :])

    def weave(gen, n, r0, nrows, every, free, due=None):
        todo = list(range(r0, r0 + nrows, SB))
        for _ in range(free):
            ln1_chunk(todo.pop(0), SB)
        for j in range(n):
            acc = next(gen)
            if todo and j % every == 0:
                ln1_chunk(todo.pop(0), SB, acc, due)
        assert not todo

    def proj_gen(tile, col0, store):
        lane_t = lax.broadcasted_iota(jnp.int32, (T, 128), 1)
        tiles = []
        done = 0
        for n in range(KT):
            acc = None
            for k in range(KT):
                p = jnp.dot(ln1_tile(tile, k),
                            wqkv_ref[k * 128:(k + 1) * 128, col0 + n * 128:col0 + (n + 1) * 128],
                            preferred_element_type=f32)
                acc = p if acc is None else p + acc
                if k == KT - 1:
                    tiles.append(acc)
                    while done < NG and (80 * done + 79) // 128 <= n:
                        lo = 80 * done
                        ta, tb = lo // 128, (lo + 79) // 128
                        a = tiles[ta]
                        if tb != ta:
                            a = jnp.where(lane_t >= lo % 128, a, tiles[tb])
                        store(done, a)
                        done += 1
                yield acc

    def k_gen(tile):
        def store(g, a):
            k_ref[g, tile * (T // 2):(tile + 1) * (T // 2), :] = _pack(a)
        return proj_gen(tile, D, store)

    def q_gen(tile):
        qscale = DH ** -0.5 * math.log2(math.e)

        def store(g, a):
            q_ref[g] = _pack(a * qscale)
        return proj_gen(tile, 0, store)

    def v_gen(tile):
        for b in range(NB):
            for hf in range(2):
                acc = None
                for k in range(KT):
                    p = lax.dot_general(wvt_ref[hf * 320:(hf + 1) * 320, k * 128:(k + 1) * 128],
                                        ln1_tile(tile, k, b * 128, 128), NT, preferred_element_type=f32)
                    acc = p if acc is None else p + acc
                    if k == KT - 1:
                        for h in range(hf * 16, hf * 16 + 16):
                            a = 8 * ((5 * h) // 2 - hf * 40)
                            if h % 2 == 0:
                                vh = [acc[a:a + 16], jnp.where(lo4, acc[a + 16:a + 24], 1.0)]
                            else:
                                vh = [jnp.where(lo4, 1.0, acc[a:a + 8]), acc[a + 8:a + 24]]
                            vt_ref[tile * NB + b, h * 24:(h + 1) * 24, :] = jnp.concatenate(vh, axis=0)
                    yield acc

    def nskip(first, b, c):
        return max(0, (W - b * 128 - c * SB) // SB) if first else 0

    def stage_qk(first, hbase, b, g):
        res = {}
        for c in [(cc + (g if first else 0)) % NH for cc in range(NH)]:
            r0 = (b * 128 + c * SB) // 2
            q0 = _mo(hbase + r0, SB // 2)
            qs = q_ref[g, r0:r0 + SB // 2, :]
            wrows = []
            for j in range(NH):
                hh = 4 * g + (j ^ c)
                mk = ((lane_h - (20 * hh) % 128) & 127) < DH
                wrows.append(jnp.where(mk, qs, zero_u))
            wc = _unpack(jnp.concatenate(wrows, axis=0))
            ns = nskip(first, b, c)
            parts = [k_ref[g, pl.ds(q0, SB // 2), :]]
            if ns < 8:
                parts.append(k_ref[g, pl.ds(q0 - (W - ns * SB) // 2, (W - ns * SB) // 2), :])
            kw = jnp.concatenate(parts, axis=0) if len(parts) > 1 else parts[0]
            s = lax.dot_general(_unpack(kw), wc, NT, preferred_element_type=f32)
            if ns == 0:
                mrg = jnp.where(tri, s[:SB], s[SB:2 * SB])
                sm = jnp.concatenate([mrg, s[2 * SB:]], axis=0)
            else:
                mrg = jnp.where(tri, s[:SB], NEG)
                sm = jnp.concatenate([mrg, s[SB:]], axis=0) if ns < 8 else mrg
            m = jnp.max(jnp.max(sm.reshape(sm.shape[0] // 8, 8, 128), axis=0), axis=0, keepdims=True)
            res[c] = (sm, m)
        return res

    def sel(mk, hi, lo):
        if lo is None and hi is None:
            return None
        return jnp.where(mk, zero_u if hi is None else hi, zero_u if lo is None else lo)

    def stage_exp(first, b, sres, toks, gate):
        pm = [jnp.exp2(sres[c][0][:SB] - sres[c][1]) for c in range(NH)]
        rho0 = max(0, 8 - 4 * b) if first else 0
        pw = [{} for _ in range(NH)]
        blks = [[] for _ in range(NH)]
        for rho in range(rho0, 12):
            cur = []
            for c in range(NH):
                ns = nskip(first, b, c)
                sm, m = sres[c]
                j = rho - c
                if j < ns or j >= NBLK:
                    cur.append(None)
                elif j == NBLK - 1:
                    cur.append(_pack(jnp.where(tri, pm[c], 0.0) if ns == 0 else pm[c]))
                elif j == 0:
                    cur.append(_pack(jnp.where(tri, 0.0, pm[c])))
                else:
                    r0 = (j - ns + (1 if ns else 0)) * SB
                    if toks:
                        ntok = len(toks) * 32
                        pos = gate[0] + ((rho - rho0) * (ntok - gate[0] - gate[1])) // (12 - rho0)
                        tok = toks[pos // 32][(pos % 32) * 8:(pos % 32) * 8 + 8]
                        mg = jnp.where(never8, tok, jnp.broadcast_to(m, (8, 128)))
                        d = (sm[r0:r0 + SB].reshape(4, 8, 128) - mg[None]).reshape(SB, 128)
                    else:
                        d = sm[r0:r0 + SB] - m
                    cur.append(_pack(jnp.exp2(d)))
            cur = [sel(mk1, cur[e ^ 1], cur[e]) for e in range(NH)]
            cur = [sel(mk2, cur[e ^ 2], cur[e]) for e in range(NH)]
            for e in range(NH):
                blks[e].append(cur[e])
                if rho % 4 == 3:
                    pw[e][rho // 4] = _unpack(jnp.concatenate(blks[e], axis=0))
                    blks[e] = []
        return pw

    def stage_pv(blk, b, g, pw, after):
        vb = blk + b - 2
        res = [None] * NH
        for t in range(3):
            if t in pw[0]:
                for e in range(NH):
                    h = 4 * g + e
                    r = lax.dot_general(vt_ref[vb + t, h * 24:(h + 1) * 24, :], pw[e][t], NN,
                                        precision=lax.Precision.DEFAULT, preferred_element_type=f32)
                    res[e] = r if res[e] is None else r + res[e]
            after(t)
        rws = []
        for e in (0, 2):
            ev, od = res[e], res[e + 1]
            inv = 1.0 / jnp.where(lo4, od[0:8], ev[16:24])
            rol = pltpu.roll(inv, 4, 0)
            inv_e = jnp.where(lo4, rol, inv)
            inv_o = jnp.where(lo4, inv, rol)
            rws += [ev[0:8] * inv_e, ev[8:16] * inv_e, jnp.where(lo4, ev[16:24], od[0:8]) * rol,
                    od[8:16] * inv_o, od[16:24] * inv_o]
        ot_ref[g * 80:(g + 1) * 80, b * 128:(b + 1) * 128] = jnp.concatenate(rws, axis=0)

    def attention(first, tile, gen, lag, fills, gate):
        units = [(b, g) for b in range(NB) for g in range(NG)]
        pws = []
        for u in range(len(units) + lag):
            if u < len(units):
                sres = stage_qk(first, tile * (T // 2), *units[u])
            toks = []
            fill = fills[0] if u < fills[1] else fills[2]

            def after(t):
                v = _pull(gen, fill[t])
                if v is not None and len(toks) < gate[2]:
                    toks.append(v)
            if u >= lag:
                stage_pv(tile * NB, *units[u - lag], pws[u - lag], after)
            else:
                for t in range(3):
                    after(t)
            if u < len(units):
                pws.append(stage_exp(first, units[u][0], sres, toks, gate))

    def out_proj(base, split):
        o_t = ot_ref[...].T
        lhs = []
        for t in range(KT):
            e_lane = ((lane_h + t * 128) // DH) % NH
            ob = _pack(o_t[:, t * 128:(t + 1) * 128])
            blks = [ob[r * 16:(r + 1) * 16, :] for r in range(T // SB)]
            for bit in (1, 2):
                mk = (e_lane & bit) != 0
                blks = [jnp.where(mk, blks[r ^ bit], blks[r]) for r in range(T // SB)]
            lhs.append(_unpack(jnp.concatenate(blks, axis=0)))
        outs = []
        cnt = 0
        for n in range(KT):
            acc = x_ref[pl.ds(base, T), n * 128:(n + 1) * 128].astype(f32)
            for k in range(KT):
                w = wo_ref[k * 128:(k + 1) * 128, n * 128:(n + 1) * 128]
                if cnt < len(split):
                    m = T // split[cnt]
                    acc = jnp.concatenate(
                        [jnp.dot(lhs[k][r:r + m], w, preferred_element_type=f32) + acc[r:r + m]
                         for r in range(0, T, m)], axis=0)
                else:
                    acc = jnp.dot(lhs[k], w, preferred_element_type=f32) + acc
                cnt += 1
            outs.append(acc)
        return jnp.concatenate(outs, axis=1)

    def finish(hres, gen, pace):
        toks = []
        while True:
            v = _pull(gen, 4)
            if v is None:
                break
            toks.append(v)
        h_ref[...] = hres
        for c, r in enumerate(range(0, T, SB)):
            pos = pace[0] + c * pace[1]
            tok = toks[pos // 8][(pos % 8) * SB:(pos % 8 + 1) * SB]
            ln2_ref[r:r + SB, :] = _ln(after_tok(hres[r:r + SB], tok)).astype(bf16)

    def ffn_gen(tile, done=None):
        ln2 = [ln2_ref[:, k * 128:(k + 1) * 128] for k in range(KT)]
        acts = []

        def proj(w_ref, r0):
            acc = None
            for k in range(KT):
                p = lax.dot_general(ln2[k], w_ref[r0:r0 + 128, k * 128:(k + 1) * 128], NT,
                                    preferred_element_type=f32)
                acc = p if acc is None else p + acc
                if k == KT - 1:
                    res.append(acc)
                yield acc

        for j in range(FT):
            res = []
            yield from proj(wg_ref, j * 128)
            yield from proj(wu_ref, j * 128)
            acts.append(_sigmoid(res[0]) * res[1])
        res = []
        yield from proj(wt_ref, 0)
        acts.append((_sigmoid(res[0]) * pltpu.roll(res[0], FR, 1))[:, :FR])
        cache = {}

        def act(j, ra, nr):
            if (j, ra, nr) not in cache:
                cache[j, ra, nr] = acts[j][ra:ra + nr].astype(bf16)
            return cache[j, ra, nr]

        pieces = [(n, 0, T) for n in range(KT)]
        if done is not None:
            pieces = pieces[:-1] + [(KT - 1, 0, T - LAST_ROWS), (KT - 1, T - LAST_ROWS, LAST_ROWS)]
        for idx, (n, ra, nr) in enumerate(pieces):
            acc = h_ref[ra:ra + nr, n * 128:(n + 1) * 128]
            for j in range(FT + 1):
                r1 = min(F, (j + 1) * 128)
                acc = jnp.dot(act(j, ra, nr), wd_ref[j * 128:r1, n * 128:(n + 1) * 128],
                              preferred_element_type=f32) + acc
                if j == FT:
                    o_ref[pl.ds(_mo(tile * T + ra, 16), nr), n * 128:(n + 1) * 128] = acc.astype(o_ref.dtype)
                    if done is not None:
                        done(idx, n, ra, nr)
                yield acc

    def ocopy(tile):
        r0 = _mo(tile * T, T)
        return pltpu.make_async_copy(rows(o_ref, r0, T), rows(o_hbm, r0, T), osem.at[tile])

    def ocopy_last(idx, n, ra, nr):
        sl = (pl.ds(S - T + ra, nr), pl.ds(n * 128, 128))
        return pltpu.make_async_copy(o_ref.at[sl], o_hbm.at[sl], osem.at[NTILE - 1 + idx])

    def prologue():
        ka = 128 * KSPLIT
        cp_x0, cp_x1 = xcopy(0, T, 0), xcopy(T, T, 1)
        cp_ka, cp_kb = wcopy(D, ka, 2), wcopy(D + ka, D - ka, 3)
        cp_v, cp_q = wcopy(2 * D, D, 4), wcopy(0, D, 5)
        cp_o = copy(wo_hbm, wo_ref, 6)
        cp_ffn = [copy(rows(wg_hbm, 0, FT * 128), wg_ref, 7), copy(rows(wu_hbm, 0, FT * 128), wu_ref, 8),
                  copy(rows(wg_hbm, FT * 128, FR), rows(wt_ref, 0, FR), 9),
                  copy(rows(wu_hbm, FT * 128, FR), rows(wt_ref, FR, FR), 10),
                  copy(wd_hbm, wd_ref, 11)]
        cp_xs = [xcopy(2 * T * (j + 1), 2 * T, 12 + j) for j in range(3)]
        for cp in [cp_x0, cp_x1, cp_ka, cp_kb, cp_xs[0], cp_v, cp_xs[1], cp_q, cp_xs[2], cp_o] + cp_ffn:
            cp.start()
        cp_x0.wait()
        ln1_chunk(0, T)
        cp_x1.wait()
        ln1_chunk(T, T)
        g0, g1, g6 = k_gen(0), k_gen(1), k_gen(6)
        gen = _chain(_take(g0, KSPLIT * KT), _take(g1, KSPLIT * KT), g0, g1, k_gen(2), k_gen(3),
                     v_gen(0), v_gen(1), k_gen(4), k_gen(5), v_gen(2), v_gen(3), q_gen(0),
                     _take(g6, 1), v_gen(4), v_gen(5), v_gen(6), v_gen(7), g6, k_gen(7))
        n1, n2, n3, n4 = REGIONS
        cp_ka.wait()
        _pull(gen, n1)
        cp_kb.wait()
        _pull(gen, n2)
        cp_xs[0].wait()
        left = 50 - n1 - n2
        weave(gen, left, 2 * T, T, 2, 2)
        weave(gen, 25, 3 * T, T, 3, 0)
        _pull(gen, n3 - left - 25)
        cp_v.wait()
        cp_xs[1].wait()
        wvt_ref[...] = wqkv_ref[:, 2 * D:].T
        left = 100 - n1 - n2 - n3
        _pull(gen, left)
        weave(gen, 40, 4 * T, T, 4, 0, LN1_DUE)
        weave(gen, 25, 5 * T, T, 3, 0, LN1_DUE)
        _pull(gen, n4 - left - 65)
        cp_q.wait()
        cp_xs[2].wait()
        cp_o.wait()
        left = 230 - n1 - n2 - n3 - n4
        weave(gen, left + 25, 6 * T, 2 * T, 4, 0, LN1_DUE)
        _pull(gen, PRE0)
        attention(True, 0, gen, LAG0, FILL0, GATE0)
        _pull(gen, TAIL0[0])
        finish(out_proj(0, TAIL0[1]), gen, PACE0)
        for cp in cp_ffn:
            cp.wait()

    def body(i, carry):
        _pull(q_gen(i), 100)
        gen = ffn_gen(i - 1)
        _pull(gen, PRE)
        attention(False, i, gen, LAG, FILL, GATE)
        _pull(gen, TAIL[0])
        finish(out_proj(pl.multiple_of(i * T, T), TAIL[1]), gen, PACE)
        ocopy(i - 1).start()
        return carry

    def epilogue():
        cps = []

        def done(*a):
            cps.append(ocopy_last(*a))
            cps[-1].start()
        _pull(ffn_gen(NTILE - 1, done), 1000)
        for t in range(NTILE - 1):
            ocopy(t).wait()
        for cp in cps:
            cp.wait()

    @pl.when(step == 0)
    def _():
        prologue()
        lax.fori_loop(1, NTILE, body, 0)
        epilogue()


@jax.jit
def pallas_sequential_preLN__sliding_block__glu_gated_glu__prompt_kernel(
    A_x: jax.Array,
    A_wqkv: jax.Array,
    A_wo: jax.Array,
    B_x: jax.Array,
    B_w_gate: jax.Array,
    B_w_up: jax.Array,
    B_w_down: jax.Array,
):
    del B_x
    anyspec = pl.BlockSpec(memory_space=pl.ANY)
    out = pl.pallas_call(
        _kernel,
        grid=(2,),
        in_specs=[anyspec] * 6,
        out_specs=anyspec,
        out_shape=jax.ShapeDtypeStruct((S, D), bf16),
        scratch_shapes=[
            pltpu.VMEM((S, D), bf16),
            pltpu.VMEM((D, 3 * D), bf16),
            pltpu.VMEM((D, D), bf16),
            pltpu.VMEM((FT * 128, D), bf16),
            pltpu.VMEM((FT * 128, D), bf16),
            pltpu.VMEM((2 * FR, D), bf16),
            pltpu.VMEM((F, D), bf16),
            pltpu.SemaphoreType.DMA((15,)),
            pltpu.VMEM((D, D), bf16),
            pltpu.VMEM((NG, S // 2, 128), u32),
            pltpu.VMEM((S // 128, H * 24, 128), f32),
            pltpu.VMEM((NG, T // 2, 128), u32),
            pltpu.VMEM((D, T), f32),
            pltpu.VMEM((KT, S, 128), bf16),
            pltpu.VMEM((T, D), bf16),
            pltpu.VMEM((T, D), f32),
            pltpu.VMEM((S, D), bf16),
            pltpu.SemaphoreType.DMA((NTILE + KT,)),
        ],
        compiler_params=pltpu.CompilerParams(dimension_semantics=("arbitrary",),
                                             vmem_limit_bytes=100 * 1024 * 1024),
    )(A_x.reshape(S, D), A_wqkv, A_wo, B_w_gate.T, B_w_up.T, B_w_down)
    return out.reshape(1, S, D)
```
